```python
import jax
import jax.numpy as jnp

def _softmax(x, axis=-1):
    return jax.nn.softmax(x, axis=axis)

def _gelu(x):
    return jax.nn.gelu(x, approximate=True)

def _silu(x):
    return jax.nn.silu(x)

def _sigmoid(x):
    return jax.nn.sigmoid(x)

def _layernorm(x, axis=-1, eps=1e-05):
    m = jnp.mean(x, axis=axis, keepdims=True)
    v = jnp.var(x, axis=axis, keepdims=True)
    return (x - m) / jnp.sqrt(v + eps)

def _scatter_add(tgt, idx, src, axis=0):
    return tgt.at[idx].add(src)

def _segment_sum(src, seg, n):
    return jax.ops.segment_sum(src, seg, n)

class _Rng:

    def __init__(self, key):
        self._k = key

    def _next(self):
        self._k, sub = jax.random.split(self._k)
        return sub

    def normal(self, shape):
        return jax.random.normal(self._next(), shape, dtype=jnp.bfloat16)

    def randint(self, lo, hi, shape):
        return jax.random.randint(self._next(), shape, lo, hi, dtype=jnp.int32)

    def uniform(self, shape, lo=0.0, hi=1.0):
        return jax.random.uniform(self._next(), shape, jnp.bfloat16, lo, hi)

    def permutation(self, n):
        return jax.random.permutation(self._next(), n)
kernel_name = 'gated_mix__memory_aug_recurrent_mem_tr__mixer_s_mlp__prompt'

def setup_inputs():
    _rng = _Rng(jax.random.key(int.from_bytes(__import__("os").urandom(4), "little")))
    _w = lambda a: (lambda t: t.astype(jnp.bfloat16) if jnp.issubdtype(t.dtype, jnp.floating) else t)(jnp.asarray(a))

    def _A_setup():
        B, S, Dm = (1, 2048, 1024)
        H, Dh = (32, 128)
        M, seg = (8, 32)
        seg = min(seg, S)
        S = S // seg * seg
        return {'x': _w((lambda *s: _rng.normal(s) * 0.05)(B, S, Dm)), 'mem0': _w((lambda *s: _rng.normal(s) * 0.05)(B, M, Dm)), 'Wq': _w((lambda *s: _rng.normal(s) * 0.05)(Dm, H, Dh) * Dm ** (-0.5)), 'Wk': _w((lambda *s: _rng.normal(s) * 0.05)(Dm, H, Dh) * Dm ** (-0.5)), 'Wv': _w((lambda *s: _rng.normal(s) * 0.05)(Dm, H, Dh) * Dm ** (-0.5)), 'Wo': _w((lambda *s: _rng.normal(s) * 0.05)(H, Dh, Dm) * (H * Dh) ** (-0.5)), 'seg_len': seg}
    _A_in = _A_setup()

    def _B_setup():
        B, S, D, F = (1, 2048, 1024, 3584)
        return {'x': _w((lambda *s: _rng.normal(s) * 0.05)(B, S, D)), 'w1': _w((lambda *s: _rng.normal(s) * 0.05)(D, D) * D ** (-0.5)), 'w2': _w((lambda *s: _rng.normal(s) * 0.05)(D, D) * D ** (-0.5)), 'w3': _w((lambda *s: _rng.normal(s) * 0.05)(D, F) * D ** (-0.5)), 'w4': _w((lambda *s: _rng.normal(s) * 0.05)(F, D) * F ** (-0.5))}
    _B_in = _B_setup()
    return {'A_x': _A_in['x'], 'A_mem0': _A_in['mem0'], 'A_Wq': _A_in['Wq'], 'A_Wk': _A_in['Wk'], 'A_Wv': _A_in['Wv'], 'A_Wo': _A_in['Wo'], 'A_seg_len': _A_in['seg_len'], 'B_x': _B_in['x'], 'B_w1': _B_in['w1'], 'B_w2': _B_in['w2'], 'B_w3': _B_in['w3'], 'B_w4': _B_in['w4'], 'gate_w': _w((lambda *s: _rng.normal(s) * 0.05)(1024))}

def reference(A_x, A_mem0, A_Wq, A_Wk, A_Wv, A_Wo, A_seg_len, B_x, B_w1, B_w2, B_w3, B_w4, gate_w):

    def _A_ref(x, mem0, Wq, Wk, Wv, Wo, seg_len):
        B, S, Dm = x.shape
        H, Dh = (Wq.shape[1], Wq.shape[2])
        M = mem0.shape[1]
        scale = Dh ** (-0.5)
        n_seg = S // seg_len
        L = M + seg_len
        idx = jnp.arange(L)
        mask = (idx[:, None] < M) | (idx[:, None] >= idx[None, :])
        mem = mem0
        outs = []
        for s in range(n_seg):
            xs = x[:, s * seg_len:(s + 1) * seg_len, :].copy()
            h = jnp.concatenate([mem, xs], axis=1)
            q = jnp.einsum('btd,dhe->bhte', h, Wq)
            k = jnp.einsum('btd,dhe->bhte', h, Wk)
            v = jnp.einsum('btd,dhe->bhte', h, Wv)
            scores = jnp.einsum('bhqe,bhke->bhqk', q, k) * scale
            scores = jnp.where(mask[None, None], scores, -1000000000.0)
            p = _softmax(scores, axis=-1)
            o = jnp.einsum('bhqk,bhke->bhqe', p, v)
            o = jnp.einsum('bhte,hed->btd', o, Wo)
            mem = o[:, :M, :].copy()
            outs.append(o[:, M:, :])
        return jnp.concatenate(outs, axis=1)

    def _B_ref(x, w1, w2, w3, w4):
        B, S, D = x.shape
        h = _gelu(_layernorm(x, axis=-1) @ w1)
        c = D // 4
        g0 = jnp.pad(h[:, :, 0 * c:1 * c], ((0, 0), (1, 0), (0, 0)))[:, :S, :]
        g1 = jnp.pad(h[:, :, 1 * c:2 * c], ((0, 0), (0, 1), (0, 0)))[:, 1:, :]
        g2 = jnp.pad(h[:, :, 2 * c:3 * c], ((0, 0), (2, 0), (0, 0)))[:, :S, :]
        g3 = jnp.pad(h[:, :, 3 * c:], ((0, 0), (0, 2), (0, 0)))[:, 2:, :]
        hs = jnp.concatenate([g0, g1, g2, g3], axis=-1) @ w2
        x1 = x + hs
        h2 = _gelu(_layernorm(x1, axis=-1) @ w3) @ w4
        return x1 + h2
    x = A_x
    g = _sigmoid((x * gate_w).sum(-1, keepdims=True))
    a = _A_ref(x, A_mem0, A_Wq, A_Wk, A_Wv, A_Wo, A_seg_len)
    b = _B_ref(x, B_w1, B_w2, B_w3, B_w4)
    return g * a + (1 - g) * b
```

```python
import functools

import jax
import jax.numpy as jnp
from jax import lax
import jax.experimental.pallas as pl
import jax.experimental.pallas.tpu as pltpu

F32, BF16, U32 = jnp.float32, jnp.bfloat16, jnp.uint32
LANE = 128
PAD = 8


def _layernorm(x, eps=1e-5):
    m = jnp.mean(x, axis=-1, keepdims=True)
    c = x - m
    v = jnp.mean(c * c, axis=-1, keepdims=True)
    return c * lax.rsqrt(v + eps)


def _gelu(x):
    return jax.nn.gelu(x, approximate=True)


def _dot(a, b):
    return jnp.dot(a, b, preferred_element_type=F32)


def _transpose8(v, masks):
    v = list(v)
    for k, m in zip((1, 2, 4), masks):
        nv = list(v)
        for r in range(8):
            if r & k:
                continue
            a, b = v[r], v[r | k]
            nv[r] = jnp.where(m, a, pltpu.roll(b, k, 0))
            nv[r | k] = jnp.where(m, pltpu.roll(a, 8 - k, 0), b)
        v = nv
    return v


def _kernel(ax_hbm, mem_hbm, wq_hbm, wk_hbm, wv_hbm, wo_hbm,
            w1_hbm, w2_hbm, w3_hbm, w4_hbm, gw_ref,
            out_hbm,
            ax, mem0, w1, w2, w3, w4, wo, wqkv, stage, hbuf, ybuf, bbuf, gbuf, obuf,
            sems, stage_sems, *, seg, n_heads, tm1, tm3, skew):
    S, D = ax.shape
    F = w3.shape[1]
    M = mem0.shape[0]
    E = LANE
    H = n_heads
    L = M + seg
    ND = D // LANE

    def copy(src, dst, i):
        return pltpu.make_async_copy(src, dst, sems.at[i])

    cp_bx = [copy(ax_hbm.at[pl.ds(i * tm1, tm1)], ax.at[pl.ds(i * tm1, tm1)], i) for i in range(S // tm1)]
    n0 = S // tm1
    cp_w1 = copy(w1_hbm, w1, n0)
    cp_w2 = copy(w2_hbm, w2, n0 + 1)
    cp_w3 = copy(w3_hbm, w3, n0 + 2)
    cp_w4 = copy(w4_hbm, w4, n0 + 3)
    cp_mem = copy(mem_hbm, mem0, n0 + 5)
    cp_wo = [copy(wo_hbm.at[:, pl.ds(c * LANE, LANE)], wo.at[c], n0 + 6) for c in range(ND)]
    out_sem = sems.at[n0 + 7]

    n3 = S // tm3
    dch = D // n3

    def cp_stage(i, slot):
        return [pltpu.make_async_copy(w.at[pl.ds(pl.multiple_of(i * (dch * H), dch * H), dch * H)],
                                      stage.at[slot, t], stage_sems.at[slot, t])
                for t, w in enumerate((wq_hbm, wk_hbm, wv_hbm))]

    cp_bx[0].start()
    cp_w1.start()
    zpad = jnp.zeros((PAD, LANE), F32)
    for c in range(ND):
        hbuf[c, pl.ds(0, PAD), :] = zpad
        hbuf[c, pl.ds(PAD + S, PAD), :] = zpad
    cp_bx[0].wait()
    cp_w1.wait()
    for cp in cp_bx[1:]:
        cp.start()
    cp_w2.start()
    cp_w3.start()
    cp_w4.start()

    for i in range(S // tm1):
        if i > 0:
            cp_bx[i].wait()
        x = ax[pl.ds(i * tm1, tm1), :].astype(F32)
        h = _gelu(_dot(_layernorm(x).astype(BF16), w1[...]))
        for c in range(ND):
            hbuf[c, pl.ds(PAD + i * tm1, tm1), :] = h[:, c * LANE:(c + 1) * LANE]

    cp_w2.wait()
    cp_mem.start()
    for cp in cp_stage(0, 0):
        cp.start()
    shifts = (-1, 1, -2, 2)

    def b2_body(i, carry):
        r0 = pl.multiple_of(i * tm1, tm1)
        cols = []
        for c in range(ND):
            win = hbuf.at[c, pl.ds(r0, tm1 + 2 * PAD)]
            cols.append(win[pl.ds(PAD + shifts[c * 4 // ND], tm1), :].astype(BF16))
        g = jnp.concatenate(cols, axis=1)
        x1 = ax[pl.ds(r0, tm1), :].astype(F32) + _dot(g, w2[...])
        bbuf[pl.ds(r0, tm1), :] = x1
        ybuf[pl.ds(r0, tm1), :] = _layernorm(x1).astype(BF16)
        return carry

    lax.fori_loop(0, S // tm1, b2_body, 0)

    cp_w3.wait()
    cp_w4.wait()
    for cp in cp_wo:
        cp.start()
    gw = gw_ref[...].astype(F32)
    sub = lax.broadcasted_iota(jnp.int32, (8, LANE), 0)
    masks = [(sub & k) == 0 for k in (1, 2, 4)]

    def b3_body(i, carry):
        slot = i % 2

        @pl.when(i + 1 < n3)
        def _():
            for cp in cp_stage(i + 1, 1 - slot):
                cp.start()

        for cp in cp_stage(i, slot):
            cp.wait()

        r0 = pl.multiple_of(i * tm3, tm3)
        y = ybuf[pl.ds(r0, tm3), :]
        u = _gelu(_dot(y, w3[...])).astype(BF16)
        b = bbuf[pl.ds(r0, tm3), :] + _dot(u, w4[...])
        xa = ax[pl.ds(r0, tm3), :].astype(F32)
        gate = jax.nn.sigmoid(jnp.sum(xa * gw, axis=-1, keepdims=True))
        bbuf[pl.ds(r0, tm3), :] = (1.0 - gate) * b
        gbuf[pl.ds(r0, tm3), :] = jnp.broadcast_to(gate, (tm3, LANE))

        for t in range(3):
            src = stage.at[slot, t].bitcast(U32)
            for g16 in range(dch // 16):
                for half in range(H // 16):
                    los, his = [], []
                    for r in range(8):
                        base = (g16 * 16 + 2 * r) * (H // 2) + half * 8
                        e = src[pl.ds(base, 8), :]
                        o = src[pl.ds(base + H // 2, 8), :]
                        los.append((e & U32(0xFFFF)) | (o << 16))
                        his.append((e >> 16) | (o & U32(0xFFFF0000)))
                    los, his = _transpose8(los, masks), _transpose8(his, masks)
                    dst = pl.ds(pl.multiple_of(i * (dch // 2) + g16 * 8, 8), 8)
                    for j in range(8):
                        hd = 2 * (half * 8 + j)
                        wqkv[hd * 3 + t, dst, :] = los[j]
                        wqkv[(hd + 1) * 3 + t, dst, :] = his[j]
        return carry

    lax.fori_loop(0, n3, b3_body, 0)

    cp_mem.wait()
    for cp in cp_wo:
        cp.wait()
    scale = E ** -0.5
    row = lax.broadcasted_iota(jnp.int32, (L, L), 0)
    col = lax.broadcasted_iota(jnp.int32, (L, L), 1)
    allow = (row < M) | (row >= col)
    wo32 = wo.bitcast(U32)

    def a_body(s, mem):
        r0 = pl.multiple_of(s * seg, seg)
        hin = jnp.concatenate([mem, ax[pl.ds(r0, seg), :].astype(F32)], axis=0)

        def proj(hd):
            w = jnp.concatenate([pltpu.bitcast(wqkv[hd * 3 + t], BF16) for t in range(3)], axis=1)
            y = _dot(hin, w)
            return y[:, :E], y[:, E:2 * E], y[:, 2 * E:]

        def attend(q, k, v):
            sc = lax.dot_general(q, k, (((1,), (1,)), ((), ())), preferred_element_type=F32) * scale
            sc = jnp.where(allow, sc, -1e9)
            p = jnp.exp(sc - jnp.max(sc, axis=-1, keepdims=True))
            p = p / jnp.sum(p, axis=-1, keepdims=True)
            return _dot(p, v)

        pending, heads = {}, []
        for hd in range(H + skew):
            if hd < H:
                pending[hd] = proj(hd)
            if hd >= skew:
                heads.append(attend(*pending.pop(hd - skew)))
        o = jnp.concatenate(heads, axis=1)
        w = jnp.concatenate([pltpu.bitcast(wo32[c], BF16) for c in range(ND)], axis=1)
        res = _dot(o, w)
        gate = gbuf[pl.ds(r0, seg), :]
        gate = jnp.concatenate([gate] * ND, axis=1)
        obuf[pl.ds(r0, seg), :] = (gate * res[M:] + bbuf[pl.ds(r0, seg), :]).astype(obuf.dtype)
        pltpu.make_async_copy(obuf.at[pl.ds(r0, seg)], out_hbm.at[pl.ds(r0, seg)], out_sem).start()
        return res[:M]

    lax.fori_loop(0, S // seg, a_body, mem0[...].astype(F32))
    pltpu.make_async_copy(obuf, out_hbm, out_sem).wait()


@functools.partial(jax.jit, static_argnames=("A_seg_len",))
def pallas_gated_mix__memory_aug_recurrent_mem_tr__mixer_s_mlp__prompt_kernel(
    A_x: jax.Array,
    A_mem0: jax.Array,
    A_Wq: jax.Array,
    A_Wk: jax.Array,
    A_Wv: jax.Array,
    A_Wo: jax.Array,
    A_seg_len: int,
    B_x: jax.Array,
    B_w1: jax.Array,
    B_w2: jax.Array,
    B_w3: jax.Array,
    B_w4: jax.Array,
    gate_w: jax.Array,
):
    B, S, D = A_x.shape
    M = A_mem0.shape[1]
    _, H, E = A_Wq.shape
    F = B_w3.shape[1]
    seg = int(A_seg_len)
    assert B == 1 and E == LANE and S % seg == 0 and D % (4 * LANE) == 0 and H % 16 == 0
    tm1, tm3, skew = 512, 256, 4
    nd = D // LANE
    dch = D // (S // tm3)

    hbm = pl.BlockSpec(memory_space=pl.ANY)
    out = pl.pallas_call(
        functools.partial(_kernel, seg=seg, n_heads=H, tm1=tm1, tm3=tm3, skew=skew),
        out_shape=jax.ShapeDtypeStruct((S, D), A_x.dtype),
        in_specs=[hbm] * 10 + [pl.BlockSpec(memory_space=pltpu.VMEM)],
        out_specs=hbm,
        scratch_shapes=[
            pltpu.VMEM((S, D), BF16),
            pltpu.VMEM((M, D), BF16),
            pltpu.VMEM((D, D), BF16),
            pltpu.VMEM((D, D), BF16),
            pltpu.VMEM((D, F), BF16),
            pltpu.VMEM((F, D), BF16),
            pltpu.VMEM((nd, H * E, LANE), BF16),
            pltpu.VMEM((H * 3, D // 2, LANE), U32),
            pltpu.VMEM((2, 3, dch * H, LANE), BF16),
            pltpu.VMEM((nd, S + 2 * PAD, LANE), F32),
            pltpu.VMEM((S, D), BF16),
            pltpu.VMEM((S, D), F32),
            pltpu.VMEM((S, LANE), F32),
            pltpu.VMEM((S, D), A_x.dtype),
            pltpu.SemaphoreType.DMA((S // tm1 + 8,)),
            pltpu.SemaphoreType.DMA((2, 3)),
        ],
        compiler_params=pltpu.CompilerParams(vmem_limit_bytes=124 * 1024 * 1024),
    )(
        A_x.reshape(S, D), A_mem0.reshape(M, D),
        A_Wq.reshape(D * H, E), A_Wk.reshape(D * H, E), A_Wv.reshape(D * H, E),
        A_Wo.reshape(H * E, D),
        B_w1, B_w2, B_w3, B_w4, gate_w.reshape(1, D),
    )
    return out.reshape(B, S, D)
```

```python
import functools

import jax
import jax.numpy as jnp
from jax import lax
import jax.experimental.pallas as pl
import jax.experimental.pallas.tpu as pltpu

F32, BF16, U32 = jnp.float32, jnp.bfloat16, jnp.uint32
LANE = 128
PAD = 8
HEAD_PAD = 4


def _layernorm(x, eps=1e-5):
    m = jnp.mean(x, axis=-1, keepdims=True)
    c = x - m
    v = jnp.mean(c * c, axis=-1, keepdims=True)
    return c * lax.rsqrt(v + eps)


def _gelu(x):
    return jax.nn.gelu(x, approximate=True)


def _dot(a, b):
    return jnp.dot(a, b, preferred_element_type=F32)


def _kernel(ax_hbm, mem_hbm, wq_hbm, wk_hbm, wv_hbm, wo_hbm,
            w1_hbm, w2_hbm, w3_hbm, w4_hbm, gw_hbm,
            out_hbm,
            ax, mem0, gw, w1, w2, w3, w4, wo, wqkv, stage, hbuf, ybuf, bbuf, gbuf, obuf,
            sems, stage_sems, *, seg, n_heads, cfg):
    S, D = ax.shape
    M = mem0.shape[0]
    E = LANE
    H = n_heads
    L = M + seg
    ND = D // LANE
    first, sub1, sub2, tm3, sub3 = cfg["first"], cfg["sub1"], cfg["sub2"], cfg["tm3"], cfg["sub3"]

    def copy(src, dst, i):
        return pltpu.make_async_copy(src, dst, sems.at[i])

    cp_x0 = copy(ax_hbm.at[pl.ds(0, first)], ax.at[pl.ds(0, first)], 0)
    cp_x1 = copy(ax_hbm.at[pl.ds(first, S - first)], ax.at[pl.ds(first, S - first)], 1)
    def slab_copies(src, dst, i):
        return [copy(src.at[:, pl.ds(c * LANE, LANE)], dst.at[c], i) for c in range(dst.shape[0])]

    def start(cps):
        for cp in cps:
            cp.start()

    def wait(cps):
        for cp in cps:
            cp.wait()

    def weight(ref):
        words = ref.bitcast(U32)
        return jnp.concatenate([pltpu.bitcast(words[c], BF16) for c in range(ref.shape[0])], axis=1)

    cp_w1 = slab_copies(w1_hbm, w1, 2)
    cp_w2 = slab_copies(w2_hbm, w2, 3)
    cp_w3 = slab_copies(w3_hbm, w3, 4)
    cp_w4 = slab_copies(w4_hbm, w4, 5)
    cp_mem = copy(mem_hbm, mem0, 6)
    cp_wo = slab_copies(wo_hbm, wo, 7)
    cp_gw = copy(gw_hbm, gw, 8)
    out_sem = sems.at[9]

    n3 = S // tm3
    dch = D // n3

    def cp_stage(i, slot):
        return [pltpu.make_async_copy(w.at[pl.ds(pl.multiple_of(i * (dch * H), dch * H), dch * H)],
                                      stage.at[slot, t], stage_sems.at[slot, t])
                for t, w in enumerate((wq_hbm, wk_hbm, wv_hbm))]

    def head_row(hd, t):
        return ((t * 2 + hd % 2) * (H // 2) + hd // 2) * (D // 2 + HEAD_PAD)

    cp_x0.start()
    start(cp_w1)
    zpad = jnp.zeros((PAD, LANE), F32)
    for c in range(ND):
        hbuf[c, pl.ds(0, PAD), :] = zpad
        hbuf[c, pl.ds(PAD + S, PAD), :] = zpad
    cp_x0.wait()
    wait(cp_w1)
    cp_x1.start()
    start(cp_w2)

    def b1(r0):
        x = ax[pl.ds(r0, sub1), :].astype(F32)
        h = _gelu(_dot(_layernorm(x).astype(BF16), weight(w1)))
        for c in range(ND):
            hbuf[c, pl.ds(PAD + r0, sub1), :] = h[:, c * LANE:(c + 1) * LANE]

    for r0 in range(0, first, sub1):
        b1(r0)
    cp_x1.wait()
    start(cp_w3)
    start(cp_w4)
    for r0 in range(first, S, sub1):
        b1(r0)

    wait(cp_w2)
    cp_mem.start()
    cp_gw.start()
    for cp in cp_stage(0, 0):
        cp.start()
    shifts = (-1, 1, -2, 2)
    for r0 in range(0, S, sub2):
        g = jnp.concatenate(
            [hbuf[c, pl.ds(PAD + r0 + shifts[c * 4 // ND], sub2), :].astype(BF16) for c in range(ND)], axis=1)
        x1 = ax[pl.ds(r0, sub2), :].astype(F32) + _dot(g, weight(w2))
        bbuf[pl.ds(r0, sub2), :] = x1
        ybuf[pl.ds(r0, sub2), :] = _layernorm(x1).astype(BF16)

    wait(cp_w3)
    wait(cp_w4)
    start(cp_wo)
    cp_gw.wait()
    gw8 = gw[...].astype(F32)
    gate_w = jnp.concatenate([gw8[c:c + 1, :] for c in range(ND)], axis=1)

    def b3_body(i, carry):
        slot = i % 2

        @pl.when(i + 1 < n3)
        def _():
            for cp in cp_stage(i + 1, 1 - slot):
                cp.start()

        for cp in cp_stage(i, slot):
            cp.wait()

        for j in range(tm3 // sub3):
            rows = pl.ds(pl.multiple_of(i * tm3 + j * sub3, sub3), sub3)
            u = _gelu(_dot(ybuf[rows, :], weight(w3))).astype(BF16)
            b = bbuf[rows, :] + _dot(u, weight(w4))
            gate = jax.nn.sigmoid(jnp.sum(ax[rows, :].astype(F32) * gate_w, axis=-1, keepdims=True))
            bbuf[rows, :] = (1.0 - gate) * b
            gbuf[rows, :] = jnp.broadcast_to(gate, (sub3, LANE))

        span = (H // 2 - 1) * (D // 2 + HEAD_PAD) + dch // 2
        for t in range(3):
            src = stage.at[slot, t].bitcast(U32)
            dst = [wqkv.at[pl.ds(pl.multiple_of(head_row(b, t) + i * (dch // 2), 8), span)] for b in range(2)]
            for r in range(dch // 2):
                for half in range(H // 16):
                    even = src[pl.ds(r * H + half * 8, 8), :]
                    odd = src[pl.ds(r * H + H // 2 + half * 8, 8), :]
                    rows = pl.ds(r + half * 8 * (D // 2 + HEAD_PAD), 8, stride=D // 2 + HEAD_PAD)
                    dst[0][rows, :] = (even & U32(0xFFFF)) | (odd << 16)
                    dst[1][rows, :] = (even >> 16) | (odd & U32(0xFFFF0000))
        return carry

    lax.fori_loop(0, n3, b3_body, 0)

    cp_mem.wait()
    wait(cp_wo)
    scale = E ** -0.5
    row = lax.broadcasted_iota(jnp.int32, (L, L), 0)
    col = lax.broadcasted_iota(jnp.int32, (L, L), 1)
    allow = (row < M) | (row >= col)
    wo32 = wo.bitcast(U32)
    dv, d1, d2, hs = cfg["dv"], cfg["d1"], cfg["d2"], cfg["hs"]

    def head_w(hd, t):
        return pltpu.bitcast(wqkv[pl.ds(head_row(hd, t), D // 2), :], BF16)

    def segment(s, mem):
        rows = pl.ds(pl.multiple_of(s * seg, seg), seg)
        hin = jnp.concatenate([mem, ax[rows, :].astype(F32)], axis=0)
        qk, val, prob, head_out = {}, {}, {}, {}

        def probs(hd):
            y = qk.pop(hd)
            sc = lax.dot_general(y[:, :E], y[:, E:], (((1,), (1,)), ((), ())),
                                 preferred_element_type=F32) * scale
            sc = jnp.where(allow, sc, -1e9)
            p = jnp.exp(sc - jnp.max(sc, axis=-1, keepdims=True))
            return p / jnp.sum(p, axis=-1, keepdims=True)

        def out_proj(h0, h1, c):
            o = jnp.concatenate([head_out[j] for j in range(h0, h1)], axis=1)
            return _dot(o, pltpu.bitcast(wo32[c, pl.ds(h0 * E // 2, (h1 - h0) * E // 2), :], BF16))

        early = []
        for t in range(H + dv + ND):
            if t < H:
                qk[t] = _dot(hin, jnp.concatenate([head_w(t, 0), head_w(t, 1)], axis=1))
            if 0 <= t - dv < H:
                val[t - dv] = _dot(hin, head_w(t - dv, 2))
            if t >= H + dv:
                early.append(out_proj(0, hs, t - H - dv))
            if 0 <= t - d1 < H:
                prob[t - d1] = probs(t - d1)
            if 0 <= t - dv - d2 < H:
                hd = t - dv - d2
                head_out[hd] = _dot(prob.pop(hd), val.pop(hd))
        res = jnp.concatenate([out_proj(hs, H, c) + early[c] for c in range(ND)], axis=1)
        gate = jnp.concatenate([gbuf[rows, :]] * ND, axis=1)
        obuf[rows, :] = (gate * res[M:] + bbuf[rows, :]).astype(obuf.dtype)
        pltpu.make_async_copy(obuf.at[rows], out_hbm.at[rows], out_sem).start()
        return res[:M]

    unroll = cfg["unroll"]

    def a_body(i, mem):
        for u in range(unroll):
            mem = segment(i * unroll + u, mem)
        return mem

    lax.fori_loop(0, S // seg // unroll, a_body, mem0[...].astype(F32))
    pltpu.make_async_copy(obuf, out_hbm, out_sem).wait()


CFG = dict(first=512, sub1=64, sub2=64, tm3=256, sub3=128, dv=2, d1=2, d2=3, hs=16, unroll=2)


@functools.partial(jax.jit, static_argnames=("A_seg_len",))
def pallas_gated_mix__memory_aug_recurrent_mem_tr__mixer_s_mlp__prompt_kernel(
    A_x: jax.Array,
    A_mem0: jax.Array,
    A_Wq: jax.Array,
    A_Wk: jax.Array,
    A_Wv: jax.Array,
    A_Wo: jax.Array,
    A_seg_len: int,
    B_x: jax.Array,
    B_w1: jax.Array,
    B_w2: jax.Array,
    B_w3: jax.Array,
    B_w4: jax.Array,
    gate_w: jax.Array,
):
    B, S, D = A_x.shape
    M = A_mem0.shape[1]
    _, H, E = A_Wq.shape
    F = B_w3.shape[1]
    seg = int(A_seg_len)
    assert B == 1 and E == LANE and S % seg == 0 and D % (4 * LANE) == 0 and H % 16 == 0
    nd = D // LANE
    dch = D // (S // CFG["tm3"])

    hbm = pl.BlockSpec(memory_space=pl.ANY)
    out = pl.pallas_call(
        functools.partial(_kernel, seg=seg, n_heads=H, cfg=CFG),
        out_shape=jax.ShapeDtypeStruct((S, D), A_x.dtype),
        in_specs=[hbm] * 11,
        out_specs=hbm,
        scratch_shapes=[
            pltpu.VMEM((S, D), BF16),
            pltpu.VMEM((M, D), BF16),
            pltpu.VMEM((nd, LANE), BF16),
            pltpu.VMEM((nd, D, LANE), BF16),
            pltpu.VMEM((nd, D, LANE), BF16),
            pltpu.VMEM((F // LANE, D, LANE), BF16),
            pltpu.VMEM((nd, F, LANE), BF16),
            pltpu.VMEM((nd, H * E, LANE), BF16),
            pltpu.VMEM((3 * H * (D // 2 + HEAD_PAD), LANE), U32),
            pltpu.VMEM((2, 3, dch * H, LANE), BF16),
            pltpu.VMEM((nd, S + 2 * PAD, LANE), F32),
            pltpu.VMEM((S, D), BF16),
            pltpu.VMEM((S, D), F32),
            pltpu.VMEM((S, LANE), F32),
            pltpu.VMEM((S, D), A_x.dtype),
            pltpu.SemaphoreType.DMA((10,)),
            pltpu.SemaphoreType.DMA((2, 3)),
        ],
        compiler_params=pltpu.CompilerParams(vmem_limit_bytes=124 * 1024 * 1024),
    )(
        A_x.reshape(S, D), A_mem0.reshape(M, D),
        A_Wq.reshape(D * H, E), A_Wk.reshape(D * H, E), A_Wv.reshape(D * H, E),
        A_Wo.reshape(H * E, D),
        B_w1, B_w2, B_w3, B_w4, gate_w.reshape(nd, LANE),
    )
    return out.reshape(B, S, D)
```

```python
import functools

import jax
import jax.numpy as jnp
from jax import lax
import jax.experimental.pallas as pl
import jax.experimental.pallas.tpu as pltpu

F32, BF16, U32 = jnp.float32, jnp.bfloat16, jnp.uint32
LANE = 128
PAD = 8
HEAD_PAD = 4


def _layernorm(x, eps=1e-5):
    m = jnp.mean(x, axis=-1, keepdims=True)
    c = x - m
    v = jnp.mean(c * c, axis=-1, keepdims=True)
    return c * lax.rsqrt(v + eps)


def _gelu(x):
    return jax.nn.gelu(x, approximate=True)


def _dot(a, b):
    return jnp.dot(a, b, preferred_element_type=F32)


def _kernel(ax_hbm, mem_hbm, wq_hbm, wk_hbm, wv_hbm, wo_hbm,
            w1_hbm, w2_hbm, w3_hbm, w4_hbm, gw_hbm,
            out_hbm,
            ax, mem0, gw, w1, w2, w3, w4, wo, wqkv, stage, hbuf, ybuf, bbuf, gbuf, obuf,
            sems, stage_sems, *, seg, n_heads, cfg):
    S, D = ax.shape
    M = mem0.shape[0]
    E = LANE
    H = n_heads
    L = M + seg
    ND = D // LANE
    first, sub1, sub2, tm3, sub3 = cfg["first"], cfg["sub1"], cfg["sub2"], cfg["tm3"], cfg["sub3"]

    def copy(src, dst, i):
        return pltpu.make_async_copy(src, dst, sems.at[i])

    cuts = (0, first, cfg["second"], S)
    cp_x = [copy(ax_hbm.at[pl.ds(lo, hi - lo)], ax.at[pl.ds(lo, hi - lo)], k)
            for k, (lo, hi) in enumerate(zip(cuts, cuts[1:]))]

    def slab_copies(src, dst, i):
        return [copy(src.at[:, pl.ds(c * LANE, LANE)], dst.at[c], i(c) if callable(i) else i)
                for c in range(dst.shape[0])]

    def start(cps):
        for cp in cps:
            cp.start()

    def wait(cps):
        for cp in cps:
            cp.wait()

    def weight(ref, slabs=None):
        words = ref.bitcast(U32)
        slabs = range(ref.shape[0]) if slabs is None else slabs
        return jnp.concatenate([pltpu.bitcast(words[c], BF16) for c in slabs], axis=1)

    n1 = cfg["n1"]
    cp_w1 = slab_copies(w1_hbm, w1, lambda c: 10 + (c >= n1))
    cp_w2 = slab_copies(w2_hbm, w2, 3)
    cp_w3 = slab_copies(w3_hbm, w3, 4)
    cp_w4 = slab_copies(w4_hbm, w4, 5)
    cp_mem = copy(mem_hbm, mem0, 6)
    cp_wo = slab_copies(wo_hbm, wo, 7)
    cp_gw = copy(gw_hbm, gw, 8)
    out_sem = sems.at[9]

    n3 = S // tm3
    dch = D // n3

    def cp_stage(i, slot):
        return [pltpu.make_async_copy(w.at[pl.ds(pl.multiple_of(i * (dch * H), dch * H), dch * H)],
                                      stage.at[slot, t], stage_sems.at[slot, t])
                for t, w in enumerate((wq_hbm, wk_hbm, wv_hbm))]

    def head_row(hd, t):
        return ((t * 2 + hd % 2) * (H // 2) + hd // 2) * (D // 2 + HEAD_PAD)

    for cps in (cp_x[:1], cp_w1, cp_x[1:], cp_w2, cp_w3, cp_w4, [cp_gw, cp_mem], cp_stage(0, 0)):
        start(cps)
    zpad = jnp.zeros((PAD, LANE), F32)
    for c in range(ND):
        hbuf[c, pl.ds(0, PAD), :] = zpad
        hbuf[c, pl.ds(PAD + S, PAD), :] = zpad

    def b1(y, r0, slabs):
        h = _gelu(_dot(y, weight(w1, slabs)))
        for k, c in enumerate(slabs):
            hbuf[c, pl.ds(PAD + r0, sub1), :] = h[:, k * LANE:(k + 1) * LANE]

    def normed(r0):
        return _layernorm(ax[pl.ds(r0, sub1), :].astype(F32)).astype(BF16)

    cp_x[0].wait()
    wait(cp_w1[:n1])
    for r0 in range(0, first, sub1):
        y = normed(r0)
        ybuf[pl.ds(r0, sub1), :] = y
        b1(y, r0, range(n1))
    wait(cp_w1[n1:])
    for r0 in range(0, first, sub1):
        b1(ybuf[pl.ds(r0, sub1), :], r0, range(n1, ND))
    cp_x[1].wait()
    for r0 in range(first, cuts[2], sub1):
        b1(normed(r0), r0, range(ND))
    cp_x[2].wait()
    for r0 in range(cuts[2], S, sub1):
        b1(normed(r0), r0, range(ND))

    wait(cp_w2)
    shifts = (-1, 1, -2, 2)
    for r0 in range(0, S, sub2):
        g = jnp.concatenate(
            [hbuf[c, pl.ds(PAD + r0 + shifts[c * 4 // ND], sub2), :].astype(BF16) for c in range(ND)], axis=1)
        x1 = ax[pl.ds(r0, sub2), :].astype(F32) + _dot(g, weight(w2))
        bbuf[pl.ds(r0, sub2), :] = x1
        ybuf[pl.ds(r0, sub2), :] = _layernorm(x1).astype(BF16)

    wait(cp_w3)
    wait(cp_w4)
    start(cp_wo)
    cp_gw.wait()
    gw8 = gw[...].astype(F32)
    gate_w = jnp.concatenate([gw8[c:c + 1, :] for c in range(ND)], axis=1)

    def b3_body(i, carry):
        slot = i % 2

        @pl.when(i + 1 < n3)
        def _():
            start(cp_stage(i + 1, 1 - slot))

        wait(cp_stage(i, slot))

        for j in range(tm3 // sub3):
            rows = pl.ds(pl.multiple_of(i * tm3 + j * sub3, sub3), sub3)
            u = _gelu(_dot(ybuf[rows, :], weight(w3))).astype(BF16)
            b = bbuf[rows, :] + _dot(u, weight(w4))
            gate = jax.nn.sigmoid(jnp.sum(ax[rows, :].astype(F32) * gate_w, axis=-1, keepdims=True))
            bbuf[rows, :] = (1.0 - gate) * b
            gbuf[rows, :] = jnp.broadcast_to(gate, (sub3, LANE))

        span = (H // 2 - 1) * (D // 2 + HEAD_PAD) + dch // 2
        for t in range(3):
            src = stage.at[slot, t].bitcast(U32)
            dst = [wqkv.at[pl.ds(pl.multiple_of(head_row(b, t) + i * (dch // 2), 8), span)] for b in range(2)]
            for r in range(dch // 2):
                for half in range(H // 16):
                    even = src[pl.ds(r * H + half * 8, 8), :]
                    odd = src[pl.ds(r * H + H // 2 + half * 8, 8), :]
                    rows = pl.ds(r + half * 8 * (D // 2 + HEAD_PAD), 8, stride=D // 2 + HEAD_PAD)
                    dst[0][rows, :] = (even & U32(0xFFFF)) | (odd << 16)
                    dst[1][rows, :] = (even >> 16) | (odd & U32(0xFFFF0000))
        return carry

    lax.fori_loop(0, n3, b3_body, 0)

    cp_mem.wait()
    wait(cp_wo)
    scale = E ** -0.5
    row = lax.broadcasted_iota(jnp.int32, (L, L), 0)
    col = lax.broadcasted_iota(jnp.int32, (L, L), 1)
    allow = (row < M) | (row >= col)
    wo32 = wo.bitcast(U32)
    dv, d1, d2, hs = cfg["dv"], cfg["d1"], cfg["d2"], cfg["hs"]

    def head_w(hd, t):
        return pltpu.bitcast(wqkv[pl.ds(head_row(hd, t), D // 2), :], BF16)

    def segment(s, mem):
        rows = pl.ds(pl.multiple_of(s * seg, seg), seg)
        hin = jnp.concatenate([mem, ax[rows, :].astype(F32)], axis=0)
        qk, val, prob, head_out = {}, {}, {}, {}

        def probs(hd):
            y = qk.pop(hd)
            sc = lax.dot_general(y[:, :E], y[:, E:], (((1,), (1,)), ((), ())),
                                 preferred_element_type=F32) * scale
            sc = jnp.where(allow, sc, -1e9)
            p = jnp.exp(sc - jnp.max(sc, axis=-1, keepdims=True))
            return p / jnp.sum(p, axis=-1, keepdims=True)

        def out_proj(h0, h1, c):
            o = jnp.concatenate([head_out[j] for j in range(h0, h1)], axis=1)
            return _dot(o, pltpu.bitcast(wo32[c, pl.ds(h0 * E // 2, (h1 - h0) * E // 2), :], BF16))

        early = []
        for t in range(H + dv + ND):
            if t < H:
                qk[t] = _dot(hin, jnp.concatenate([head_w(t, 0), head_w(t, 1)], axis=1))
            if 0 <= t - dv < H:
                val[t - dv] = _dot(hin, head_w(t - dv, 2))
            if t >= H + dv:
                early.append(out_proj(0, hs, t - H - dv))
            if 0 <= t - d1 < H:
                prob[t - d1] = probs(t - d1)
            if 0 <= t - dv - d2 < H:
                hd = t - dv - d2
                head_out[hd] = _dot(prob.pop(hd), val.pop(hd))
        res = jnp.concatenate([out_proj(hs, H, c) + early[c] for c in range(ND)], axis=1)
        gate = jnp.concatenate([gbuf[rows, :]] * ND, axis=1)
        obuf[rows, :] = (gate * res[M:] + bbuf[rows, :]).astype(obuf.dtype)
        pltpu.make_async_copy(obuf.at[rows], out_hbm.at[rows], out_sem).start()
        return res[:M]

    unroll = cfg["unroll"]

    def a_body(i, mem):
        for u in range(unroll):
            mem = segment(i * unroll + u, mem)
        return mem

    lax.fori_loop(0, S // seg // unroll, a_body, mem0[...].astype(F32))
    pltpu.make_async_copy(obuf, out_hbm, out_sem).wait()


CFG = dict(first=384, second=1024, n1=4, sub1=64, sub2=64, tm3=256, sub3=128, dv=2, d1=2, d2=3, hs=16, unroll=2)


@functools.partial(jax.jit, static_argnames=("A_seg_len",))
def pallas_gated_mix__memory_aug_recurrent_mem_tr__mixer_s_mlp__prompt_kernel(
    A_x: jax.Array,
    A_mem0: jax.Array,
    A_Wq: jax.Array,
    A_Wk: jax.Array,
    A_Wv: jax.Array,
    A_Wo: jax.Array,
    A_seg_len: int,
    B_x: jax.Array,
    B_w1: jax.Array,
    B_w2: jax.Array,
    B_w3: jax.Array,
    B_w4: jax.Array,
    gate_w: jax.Array,
):
    B, S, D = A_x.shape
    M = A_mem0.shape[1]
    _, H, E = A_Wq.shape
    F = B_w3.shape[1]
    seg = int(A_seg_len)
    assert B == 1 and E == LANE and S % seg == 0 and D % (4 * LANE) == 0 and H % 16 == 0
    nd = D // LANE
    dch = D // (S // CFG["tm3"])

    hbm = pl.BlockSpec(memory_space=pl.ANY)
    out = pl.pallas_call(
        functools.partial(_kernel, seg=seg, n_heads=H, cfg=CFG),
        out_shape=jax.ShapeDtypeStruct((S, D), A_x.dtype),
        in_specs=[hbm] * 11,
        out_specs=hbm,
        scratch_shapes=[
            pltpu.VMEM((S, D), BF16),
            pltpu.VMEM((M, D), BF16),
            pltpu.VMEM((nd, LANE), BF16),
            pltpu.VMEM((nd, D, LANE), BF16),
            pltpu.VMEM((nd, D, LANE), BF16),
            pltpu.VMEM((F // LANE, D, LANE), BF16),
            pltpu.VMEM((nd, F, LANE), BF16),
            pltpu.VMEM((nd, H * E, LANE), BF16),
            pltpu.VMEM((3 * H * (D // 2 + HEAD_PAD), LANE), U32),
            pltpu.VMEM((2, 3, dch * H, LANE), BF16),
            pltpu.VMEM((nd, S + 2 * PAD, LANE), F32),
            pltpu.VMEM((S, D), BF16),
            pltpu.VMEM((S, D), F32),
            pltpu.VMEM((S, LANE), F32),
            pltpu.VMEM((S, D), A_x.dtype),
            pltpu.SemaphoreType.DMA((12,)),
            pltpu.SemaphoreType.DMA((2, 3)),
        ],
        compiler_params=pltpu.CompilerParams(vmem_limit_bytes=124 * 1024 * 1024),
    )(
        A_x.reshape(S, D), A_mem0.reshape(M, D),
        A_Wq.reshape(D * H, E), A_Wk.reshape(D * H, E), A_Wv.reshape(D * H, E),
        A_Wo.reshape(H * E, D),
        B_w1, B_w2, B_w3, B_w4, gate_w.reshape(nd, LANE),
    )
    return out.reshape(B, S, D)
```

```python
import functools

import jax
import jax.numpy as jnp
import numpy as np
from jax import lax
import jax.experimental.pallas as pl
import jax.experimental.pallas.tpu as pltpu

F32, BF16, U32 = jnp.float32, jnp.bfloat16, jnp.uint32
LOW16, HIGH16 = np.uint32(0xFFFF), np.uint32(0xFFFF0000)
LANE = 128
PAD = 8
HEAD_PAD = 4


def _layernorm(x, eps=1e-5):
    m = jnp.mean(x, axis=-1, keepdims=True)
    c = x - m
    v = jnp.mean(c * c, axis=-1, keepdims=True)
    return c * lax.rsqrt(v + eps)


def _gelu(x):
    return jax.nn.gelu(x, approximate=True)


def _dot(a, b):
    return jnp.dot(a, b, preferred_element_type=F32)


def _kernel(ax_hbm, mem_hbm, wq_hbm, wk_hbm, wv_hbm, wo_hbm,
            w1_hbm, w2_hbm, w3_hbm, w4_hbm, gw_hbm,
            out_hbm,
            ax, mem0, gw, w1, w2, w3, w4, wo, wqkv, stage, hbuf, ybuf, bbuf, gbuf, obuf,
            sems, stage_sems, *, seg, n_heads, cfg):
    S, D = ax.shape
    M = mem0.shape[0]
    E = LANE
    H = n_heads
    L = M + seg
    ND = D // LANE
    first, sub1, sub2, tm3, sub3 = cfg["first"], cfg["sub1"], cfg["sub2"], cfg["tm3"], cfg["sub3"]

    def copy(src, dst, i):
        return pltpu.make_async_copy(src, dst, sems.at[i])

    second = cfg["second"]
    cuts = (0, first + sub1, second + sub1, S)
    cp_x = [copy(ax_hbm.at[pl.ds(lo, hi - lo)], ax.at[pl.ds(lo, hi - lo)], k)
            for k, (lo, hi) in enumerate(zip(cuts, cuts[1:]))]

    def slab_copies(src, dst, i):
        return [copy(src.at[:, pl.ds(c * LANE, LANE)], dst.at[c], i(c) if callable(i) else i)
                for c in range(dst.shape[0])]

    def start(cps):
        for cp in cps:
            cp.start()

    def wait(cps):
        for cp in cps:
            cp.wait()

    def weight(ref, slabs=None):
        words = ref.bitcast(U32)
        slabs = range(ref.shape[0]) if slabs is None else slabs
        return jnp.concatenate([pltpu.bitcast(words[c], BF16) for c in slabs], axis=1)

    n1 = cfg["n1"]
    cp_w1 = slab_copies(w1_hbm, w1, lambda c: 10 + (c >= n1))
    cp_w2 = slab_copies(w2_hbm, w2, 3)
    cp_w3 = slab_copies(w3_hbm, w3, 4)
    cp_w4 = slab_copies(w4_hbm, w4, 5)
    cp_mem = copy(mem_hbm, mem0, 6)
    cp_wo = slab_copies(wo_hbm, wo, 7)
    cp_gw = copy(gw_hbm, gw, 8)
    out_sem = sems.at[9]

    n3 = S // tm3
    dch = D // n3

    def cp_stage(i, slot):
        return [pltpu.make_async_copy(w.at[pl.ds(pl.multiple_of(i * (dch * H), dch * H), dch * H)],
                                      stage.at[slot, t], stage_sems.at[slot, t])
                for t, w in enumerate((wq_hbm, wk_hbm, wv_hbm))]

    def head_row(hd, t):
        return ((t * 2 + hd % 2) * (H // 2) + hd // 2) * (D // 2 + HEAD_PAD)

    for cps in (cp_x[:1], cp_w1, cp_x[1:], cp_w2, cp_w3, cp_w4, [cp_gw, cp_mem], cp_stage(0, 0)):
        start(cps)
    zpad = jnp.zeros((PAD, LANE), F32)
    for c in range(ND):
        hbuf[c, pl.ds(0, PAD), :] = zpad
        hbuf[c, pl.ds(PAD + S, PAD), :] = zpad

    def b1(y, r0, slabs):
        h = _gelu(_dot(y, weight(w1, slabs)))
        for k, c in enumerate(slabs):
            hbuf[c, pl.ds(PAD + r0, sub1), :] = h[:, k * LANE:(k + 1) * LANE]

    def normed(r0):
        return _layernorm(ax[pl.ds(r0, sub1), :].astype(F32)).astype(BF16)

    def cache_normed(r0):
        ybuf[pl.ds(r0, sub1), :] = normed(r0)

    def cached(r0):
        return ybuf[pl.ds(r0, sub1), :]

    cp_x[0].wait()
    for r0 in range(0, first, sub1):
        cache_normed(r0)
    wait(cp_w1[:n1])
    for r0 in range(0, first, sub1):
        b1(cached(r0), r0, range(n1))
    wait(cp_w1[n1:])
    for r0 in range(0, first, sub1):
        b1(cached(r0), r0, range(n1, ND))
    cache_normed(first)
    cp_x[1].wait()
    for r0 in range(first, second, sub1):
        b1(cached(r0) if r0 == first else normed(r0), r0, range(ND))
    cache_normed(second)
    cp_x[2].wait()
    wait(cp_w2)
    for r0 in range(second, S, sub1):
        b1(cached(r0) if r0 == second else normed(r0), r0, range(ND))

    shifts = (-1, 1, -2, 2)
    for r0 in range(0, S, sub2):
        g = jnp.concatenate(
            [hbuf[c, pl.ds(PAD + r0 + shifts[c * 4 // ND], sub2), :].astype(BF16) for c in range(ND)], axis=1)
        x1 = ax[pl.ds(r0, sub2), :].astype(F32) + _dot(g, weight(w2))
        bbuf[pl.ds(r0, sub2), :] = x1
        ybuf[pl.ds(r0, sub2), :] = _layernorm(x1).astype(BF16)

    wait(cp_w3)
    wait(cp_w4)
    start(cp_wo)
    cp_gw.wait()
    gw8 = gw[...].astype(F32)
    gate_w = jnp.concatenate([gw8[c:c + 1, :] for c in range(ND)], axis=1)

    def b3_body(i, carry):
        slot = i % 2

        @pl.when(i + 1 < n3)
        def _():
            start(cp_stage(i + 1, 1 - slot))

        wait(cp_stage(i, slot))

        for j in range(tm3 // sub3):
            rows = pl.ds(pl.multiple_of(i * tm3 + j * sub3, sub3), sub3)
            u = _gelu(_dot(ybuf[rows, :], weight(w3))).astype(BF16)
            b = bbuf[rows, :] + _dot(u, weight(w4))
            gate = jax.nn.sigmoid(jnp.sum(ax[rows, :].astype(F32) * gate_w, axis=-1, keepdims=True))
            bbuf[rows, :] = (1.0 - gate) * b
            gbuf[rows, :] = jnp.broadcast_to(gate, (sub3, LANE))

        span = (H // 2 - 1) * (D // 2 + HEAD_PAD) + dch // 2
        for t in range(3):
            src = stage.at[slot, t].bitcast(U32)
            dst = [wqkv.at[pl.ds(pl.multiple_of(head_row(b, t) + i * (dch // 2), 8), span)] for b in range(2)]
            for r in range(dch // 2):
                for half in range(H // 16):
                    even = src[pl.ds(r * H + half * 8, 8), :]
                    odd = src[pl.ds(r * H + H // 2 + half * 8, 8), :]
                    rows = pl.ds(r + half * 8 * (D // 2 + HEAD_PAD), 8, stride=D // 2 + HEAD_PAD)
                    dst[0][rows, :] = (even & LOW16) | (odd << 16)
                    dst[1][rows, :] = (even >> 16) | (odd & HIGH16)
        return carry

    lax.fori_loop(0, n3, b3_body, 0)

    cp_mem.wait()
    wait(cp_wo)
    scale = E ** -0.5
    row = lax.broadcasted_iota(jnp.int32, (L, L), 0)
    col = lax.broadcasted_iota(jnp.int32, (L, L), 1)
    allow = (row >= seg) | (col >= seg) | (row >= col)
    wo32 = wo.bitcast(U32)
    dv, d1, d2, hs = cfg["dv"], cfg["d1"], cfg["d2"], cfg["hs"]

    def head_w(hd, t):
        return pltpu.bitcast(wqkv[pl.ds(head_row(hd, t), D // 2), :], BF16)

    def segment(s, mem):
        rows = pl.ds(pl.multiple_of(s * seg, seg), seg)
        hin = jnp.concatenate([ax[rows, :].astype(F32), mem], axis=0)
        qk, val, prob, head_out = {}, {}, {}, {}

        def probs(hd):
            y = qk.pop(hd)
            sc = lax.dot_general(y[:, :E], y[:, E:], (((1,), (1,)), ((), ())),
                                 preferred_element_type=F32) * scale
            sc = jnp.where(allow, sc, -1e9)
            p = jnp.exp(sc - jnp.max(sc, axis=-1, keepdims=True))
            return p / jnp.sum(p, axis=-1, keepdims=True)

        def out_proj(h0, h1, c):
            o = jnp.concatenate([head_out[j] for j in range(h0, h1)], axis=1)
            return _dot(o, pltpu.bitcast(wo32[c, pl.ds(h0 * E // 2, (h1 - h0) * E // 2), :], BF16))

        early = []
        for t in range(H + dv + ND):
            if t < H:
                qk[t] = _dot(hin, jnp.concatenate([head_w(t, 0), head_w(t, 1)], axis=1))
            if 0 <= t - dv < H:
                val[t - dv] = _dot(hin, head_w(t - dv, 2))
            if t >= H + dv:
                early.append(out_proj(0, hs, t - H - dv))
            if 0 <= t - d1 < H:
                prob[t - d1] = probs(t - d1)
            if 0 <= t - dv - d2 < H:
                hd = t - dv - d2
                o = _dot(prob.pop(hd), val.pop(hd))
                head_out[hd] = jnp.concatenate([o[seg:], o[:seg]], axis=0)
        res = jnp.concatenate([out_proj(hs, H, c) + early[c] for c in range(ND)], axis=1)
        gate = jnp.concatenate([gbuf[rows, :]] * ND, axis=1)
        obuf[rows, :] = (gate * res[M:] + bbuf[rows, :]).astype(obuf.dtype)
        pltpu.make_async_copy(obuf.at[rows], out_hbm.at[rows], out_sem).start()
        return res[:M]

    unroll = cfg["unroll"]

    def a_body(i, mem):
        for u in range(unroll):
            mem = segment(i * unroll + u, mem)
        return mem

    lax.fori_loop(0, S // seg // unroll, a_body, mem0[...].astype(F32))
    pltpu.make_async_copy(obuf, out_hbm, out_sem).wait()


CFG = dict(first=384, second=1024, n1=4, sub1=64, sub2=64, tm3=256, sub3=128, dv=0, d1=2, d2=5, hs=16, unroll=2)


@functools.partial(jax.jit, static_argnames=("A_seg_len",))
def pallas_gated_mix__memory_aug_recurrent_mem_tr__mixer_s_mlp__prompt_kernel(
    A_x: jax.Array,
    A_mem0: jax.Array,
    A_Wq: jax.Array,
    A_Wk: jax.Array,
    A_Wv: jax.Array,
    A_Wo: jax.Array,
    A_seg_len: int,
    B_x: jax.Array,
    B_w1: jax.Array,
    B_w2: jax.Array,
    B_w3: jax.Array,
    B_w4: jax.Array,
    gate_w: jax.Array,
):
    B, S, D = A_x.shape
    M = A_mem0.shape[1]
    _, H, E = A_Wq.shape
    F = B_w3.shape[1]
    seg = int(A_seg_len)
    assert B == 1 and E == LANE and S % seg == 0 and D % (4 * LANE) == 0 and H % 16 == 0
    nd = D // LANE
    dch = D // (S // CFG["tm3"])

    hbm = pl.BlockSpec(memory_space=pl.ANY)
    out = pl.pallas_call(
        functools.partial(_kernel, seg=seg, n_heads=H, cfg=CFG),
        out_shape=jax.ShapeDtypeStruct((S, D), A_x.dtype),
        in_specs=[hbm] * 11,
        out_specs=hbm,
        scratch_shapes=[
            pltpu.VMEM((S, D), BF16),
            pltpu.VMEM((M, D), BF16),
            pltpu.VMEM((nd, LANE), BF16),
            pltpu.VMEM((nd, D, LANE), BF16),
            pltpu.VMEM((nd, D, LANE), BF16),
            pltpu.VMEM((F // LANE, D, LANE), BF16),
            pltpu.VMEM((nd, F, LANE), BF16),
            pltpu.VMEM((nd, H * E, LANE), BF16),
            pltpu.VMEM((3 * H * (D // 2 + HEAD_PAD), LANE), U32),
            pltpu.VMEM((2, 3, dch * H, LANE), BF16),
            pltpu.VMEM((nd, S + 2 * PAD, LANE), F32),
            pltpu.VMEM((S, D), BF16),
            pltpu.VMEM((S, D), F32),
            pltpu.VMEM((S, LANE), F32),
            pltpu.VMEM((S, D), A_x.dtype),
            pltpu.SemaphoreType.DMA((12,)),
            pltpu.SemaphoreType.DMA((2, 3)),
        ],
        compiler_params=pltpu.CompilerParams(vmem_limit_bytes=124 * 1024 * 1024),
    )(
        A_x.reshape(S, D), A_mem0.reshape(M, D),
        A_Wq.reshape(D * H, E), A_Wk.reshape(D * H, E), A_Wv.reshape(D * H, E),
        A_Wo.reshape(H * E, D),
        B_w1, B_w2, B_w3, B_w4, gate_w.reshape(nd, LANE),
    )
    return out.reshape(B, S, D)
```

```python
import functools

import jax
import jax.numpy as jnp
import numpy as np
from jax import lax
import jax.experimental.pallas as pl
import jax.experimental.pallas.tpu as pltpu

F32, BF16, U32 = jnp.float32, jnp.bfloat16, jnp.uint32
LOW16, HIGH16 = np.uint32(0xFFFF), np.uint32(0xFFFF0000)
LANE = 128
PAD = 8
HEAD_PAD = 4

ROWS = 64
CUT1, CUT2 = 384, 1024
W1_FIRST = 4
B3_ROWS = 256
QK_LAG, PV_LAG = 2, 5
HEADS_EARLY = 16
UNROLL = 2


def _layernorm(x, eps=1e-5):
    m = jnp.mean(x, axis=-1, keepdims=True)
    c = x - m
    v = jnp.mean(c * c, axis=-1, keepdims=True)
    return c * lax.rsqrt(v + eps)


def _gelu(x):
    return jax.nn.gelu(x, approximate=True)


def _dot(a, b):
    return jnp.dot(a, b, preferred_element_type=F32)


def _start(copies):
    for cp in copies:
        cp.start()


def _wait(copies):
    for cp in copies:
        cp.wait()


def _weight(ref, slabs=None):
    words = ref.bitcast(U32)
    slabs = range(ref.shape[0]) if slabs is None else slabs
    return jnp.concatenate([pltpu.bitcast(words[c], BF16) for c in slabs], axis=1)


def _kernel(x_hbm, mem_hbm, wq_hbm, wk_hbm, wv_hbm, wo_hbm,
            w1_hbm, w2_hbm, w3_hbm, w4_hbm, gw_hbm,
            out_hbm,
            x, mem0, gw, w1, w2, w3, w4, wo, wqkv, stage, hbuf, ybuf, bbuf, gbuf, obuf,
            sems, stage_sems, *, seg, n_heads):
    S, D = x.shape
    M = mem0.shape[0]
    E = LANE
    H = n_heads
    ND = D // LANE

    def copy(src, dst, sem):
        return pltpu.make_async_copy(src, dst, sems.at[sem])

    def slab_copies(src, dst, slabs, sem):
        return [copy(src.at[:, pl.ds(c * LANE, LANE)], dst.at[c], sem) for c in slabs]

    cuts = (0, CUT1 + ROWS, CUT2 + ROWS, S)
    cp_x = [copy(x_hbm.at[pl.ds(lo, hi - lo)], x.at[pl.ds(lo, hi - lo)], k)
            for k, (lo, hi) in enumerate(zip(cuts, cuts[1:]))]
    cp_w1a = slab_copies(w1_hbm, w1, range(W1_FIRST), 3)
    cp_w1b = slab_copies(w1_hbm, w1, range(W1_FIRST, ND), 4)
    cp_w2 = slab_copies(w2_hbm, w2, range(ND), 5)
    cp_w3 = slab_copies(w3_hbm, w3, range(w3.shape[0]), 6)
    cp_w4 = slab_copies(w4_hbm, w4, range(ND), 7)
    cp_wo = slab_copies(wo_hbm, wo, range(ND), 8)
    cp_gw = copy(gw_hbm, gw, 9)
    cp_mem = copy(mem_hbm, mem0, 10)
    out_sem = sems.at[11]

    n3 = S // B3_ROWS
    dch = D // n3
    head_pitch = D // 2 + HEAD_PAD

    def cp_stage(i, slot):
        rows = pl.ds(pl.multiple_of(i * (dch * H), dch * H), dch * H)
        return [pltpu.make_async_copy(w.at[rows], stage.at[slot, t], stage_sems.at[slot, t])
                for t, w in enumerate((wq_hbm, wk_hbm, wv_hbm))]

    def head_row(hd, t):
        return ((t * 2 + hd % 2) * (H // 2) + hd // 2) * head_pitch

    for copies in (cp_x[:1], cp_w1a, cp_w1b, cp_x[1:], cp_w2, cp_w3, cp_w4,
                   [cp_gw, cp_mem], cp_stage(0, 0)):
        _start(copies)
    zeros = jnp.zeros((PAD, LANE), F32)
    for c in range(ND):
        hbuf[c, pl.ds(0, PAD), :] = zeros
        hbuf[c, pl.ds(PAD + S, PAD), :] = zeros

    def normed(r0):
        return _layernorm(x[pl.ds(r0, ROWS), :].astype(F32)).astype(BF16)

    def cache_normed(r0):
        ybuf[pl.ds(r0, ROWS), :] = normed(r0)

    def cached(r0):
        return ybuf[pl.ds(r0, ROWS), :]

    def b1(y, r0, slabs):
        h = _gelu(_dot(y, _weight(w1, slabs)))
        for k, c in enumerate(slabs):
            hbuf[c, pl.ds(PAD + r0, ROWS), :] = h[:, k * LANE:(k + 1) * LANE]

    cp_x[0].wait()
    for r0 in range(0, CUT1, ROWS):
        cache_normed(r0)
    _wait(cp_w1a)
    for r0 in range(0, CUT1, ROWS):
        b1(cached(r0), r0, range(W1_FIRST))
    _wait(cp_w1b)
    for r0 in range(0, CUT1, ROWS):
        b1(cached(r0), r0, range(W1_FIRST, ND))
    cache_normed(CUT1)
    cp_x[1].wait()
    for r0 in range(CUT1, CUT2, ROWS):
        b1(cached(r0) if r0 == CUT1 else normed(r0), r0, range(ND))
    cache_normed(CUT2)
    cp_x[2].wait()
    _wait(cp_w2)
    for r0 in range(CUT2, S, ROWS):
        b1(cached(r0) if r0 == CUT2 else normed(r0), r0, range(ND))

    shifts = (-1, 1, -2, 2)
    for r0 in range(0, S, ROWS):
        g = jnp.concatenate(
            [hbuf[c, pl.ds(PAD + r0 + shifts[c * 4 // ND], ROWS), :].astype(BF16) for c in range(ND)],
            axis=1)
        x1 = x[pl.ds(r0, ROWS), :].astype(F32) + _dot(g, _weight(w2))
        bbuf[pl.ds(r0, ROWS), :] = x1
        ybuf[pl.ds(r0, ROWS), :] = _layernorm(x1).astype(BF16)

    _wait(cp_w3)
    _wait(cp_w4)
    _start(cp_wo)
    cp_gw.wait()
    gw_rows = gw[...].astype(F32)
    gate_w = jnp.concatenate([gw_rows[c:c + 1, :] for c in range(ND)], axis=1)

    def b3_step(i, carry):
        slot = i % 2

        @pl.when(i + 1 < n3)
        def _():
            _start(cp_stage(i + 1, 1 - slot))

        _wait(cp_stage(i, slot))

        for j in range(B3_ROWS // ROWS):
            rows = pl.ds(pl.multiple_of(i * B3_ROWS + j * ROWS, ROWS), ROWS)
            u = _gelu(_dot(ybuf[rows, :], _weight(w3))).astype(BF16)
            b = bbuf[rows, :] + _dot(u, _weight(w4))
            gate = jax.nn.sigmoid(jnp.sum(x[rows, :].astype(F32) * gate_w, axis=-1, keepdims=True))
            bbuf[rows, :] = (1.0 - gate) * b
            gbuf[rows, :] = jnp.broadcast_to(gate, (ROWS, LANE))

        span = (H // 2 - 1) * head_pitch + dch // 2
        for t in range(3):
            src = stage.at[slot, t].bitcast(U32)
            dst = [wqkv.at[pl.ds(pl.multiple_of(head_row(hd, t) + i * (dch // 2), 8), span)]
                   for hd in range(2)]
            for r in range(dch // 2):
                for part in range(H // 16):
                    even = src[pl.ds(r * H + part * 8, 8), :]
                    odd = src[pl.ds(r * H + H // 2 + part * 8, 8), :]
                    rows = pl.ds(r + part * 8 * head_pitch, 8, stride=head_pitch)
                    dst[0][rows, :] = (even & LOW16) | (odd << 16)
                    dst[1][rows, :] = (even >> 16) | (odd & HIGH16)
        return carry

    lax.fori_loop(0, n3, b3_step, 0)

    cp_mem.wait()
    _wait(cp_wo)
    scale = E ** -0.5
    row = lax.broadcasted_iota(jnp.int32, (seg + M, seg + M), 0)
    col = lax.broadcasted_iota(jnp.int32, (seg + M, seg + M), 1)
    allow = (row >= seg) | (col >= seg) | (row >= col)
    wo_words = wo.bitcast(U32)

    def head_w(hd, t):
        return pltpu.bitcast(wqkv[pl.ds(head_row(hd, t), D // 2), :], BF16)

    def segment(s, mem):
        rows = pl.ds(pl.multiple_of(s * seg, seg), seg)
        h = jnp.concatenate([x[rows, :].astype(F32), mem], axis=0)
        qk, val, prob, head_out = {}, {}, {}, {}

        def softmax_scores(y):
            sc = lax.dot_general(y[:, :E], y[:, E:], (((1,), (1,)), ((), ())),
                                 preferred_element_type=F32) * scale
            sc = jnp.where(allow, sc, -1e9)
            p = jnp.exp(sc - jnp.max(sc, axis=-1, keepdims=True))
            return p / jnp.sum(p, axis=-1, keepdims=True)

        def out_proj(h0, h1, c):
            o = jnp.concatenate([head_out[hd] for hd in range(h0, h1)], axis=1)
            w = wo_words[c, pl.ds(h0 * E // 2, (h1 - h0) * E // 2), :]
            return _dot(o, pltpu.bitcast(w, BF16))

        early = []
        for t in range(H + ND):
            if t < H:
                qk[t] = _dot(h, jnp.concatenate([head_w(t, 0), head_w(t, 1)], axis=1))
                val[t] = _dot(h, head_w(t, 2))
            else:
                early.append(out_proj(0, HEADS_EARLY, t - H))
            if 0 <= t - QK_LAG < H:
                prob[t - QK_LAG] = softmax_scores(qk.pop(t - QK_LAG))
            if 0 <= t - PV_LAG < H:
                hd = t - PV_LAG
                o = _dot(prob.pop(hd), val.pop(hd))
                head_out[hd] = jnp.concatenate([o[seg:], o[:seg]], axis=0)
        res = jnp.concatenate([out_proj(HEADS_EARLY, H, c) + early[c] for c in range(ND)], axis=1)

        gate = jnp.concatenate([gbuf[rows, :]] * ND, axis=1)
        obuf[rows, :] = (gate * res[M:] + bbuf[rows, :]).astype(obuf.dtype)
        pltpu.make_async_copy(obuf.at[rows], out_hbm.at[rows], out_sem).start()
        return res[:M]

    def a_step(i, mem):
        for u in range(UNROLL):
            mem = segment(i * UNROLL + u, mem)
        return mem

    lax.fori_loop(0, S // seg // UNROLL, a_step, mem0[...].astype(F32))
    pltpu.make_async_copy(obuf, out_hbm, out_sem).wait()


@functools.partial(jax.jit, static_argnames=("A_seg_len",))
def pallas_gated_mix__memory_aug_recurrent_mem_tr__mixer_s_mlp__prompt_kernel(
    A_x: jax.Array,
    A_mem0: jax.Array,
    A_Wq: jax.Array,
    A_Wk: jax.Array,
    A_Wv: jax.Array,
    A_Wo: jax.Array,
    A_seg_len: int,
    B_x: jax.Array,
    B_w1: jax.Array,
    B_w2: jax.Array,
    B_w3: jax.Array,
    B_w4: jax.Array,
    gate_w: jax.Array,
):
    del B_x
    B, S, D = A_x.shape
    M = A_mem0.shape[1]
    _, H, E = A_Wq.shape
    F = B_w3.shape[1]
    seg = int(A_seg_len)
    nd = D // LANE
    dch = D // (S // B3_ROWS)
    assert B == 1 and E == LANE and D % (4 * LANE) == 0 and F % LANE == 0
    assert S % B3_ROWS == 0 and S > CUT2 + ROWS and S % (seg * UNROLL) == 0 and dch % 16 == 0
    assert seg % 16 == 0 and M % 8 == 0 and H % 16 == 0 and HEADS_EARLY + PV_LAG <= H and PV_LAG <= nd

    hbm = pl.BlockSpec(memory_space=pl.ANY)
    out = pl.pallas_call(
        functools.partial(_kernel, seg=seg, n_heads=H),
        out_shape=jax.ShapeDtypeStruct((S, D), A_x.dtype),
        in_specs=[hbm] * 11,
        out_specs=hbm,
        scratch_shapes=[
            pltpu.VMEM((S, D), BF16),
            pltpu.VMEM((M, D), BF16),
            pltpu.VMEM((nd, LANE), BF16),
            pltpu.VMEM((nd, D, LANE), BF16),
            pltpu.VMEM((nd, D, LANE), BF16),
            pltpu.VMEM((F // LANE, D, LANE), BF16),
            pltpu.VMEM((nd, F, LANE), BF16),
            pltpu.VMEM((nd, H * E, LANE), BF16),
            pltpu.VMEM((3 * H * (D // 2 + HEAD_PAD), LANE), U32),
            pltpu.VMEM((2, 3, dch * H, LANE), BF16),
            pltpu.VMEM((nd, S + 2 * PAD, LANE), F32),
            pltpu.VMEM((S, D), BF16),
            pltpu.VMEM((S, D), F32),
            pltpu.VMEM((S, LANE), F32),
            pltpu.VMEM((S, D), A_x.dtype),
            pltpu.SemaphoreType.DMA((12,)),
            pltpu.SemaphoreType.DMA((2, 3)),
        ],
        compiler_params=pltpu.CompilerParams(vmem_limit_bytes=112 * 1024 * 1024),
    )(
        A_x.reshape(S, D), A_mem0.reshape(M, D),
        A_Wq.reshape(D * H, E), A_Wk.reshape(D * H, E), A_Wv.reshape(D * H, E),
        A_Wo.reshape(H * E, D),
        B_w1, B_w2, B_w3, B_w4, gate_w.reshape(nd, LANE),
    )
    return out.reshape(B, S, D)
```

```python
import functools

import jax
import jax.numpy as jnp
import numpy as np
from jax import lax
import jax.experimental.pallas as pl
import jax.experimental.pallas.tpu as pltpu

F32, BF16, U32 = jnp.float32, jnp.bfloat16, jnp.uint32
LOW16, HIGH16 = np.uint32(0xFFFF), np.uint32(0xFFFF0000)
LANE = 128
PAD = 8
HEAD_PAD = 4

ROWS = 64
CUT1, CUT2 = 384, 1024
W1_FIRST = 4
B3_ROWS = 256
QK_LAG, PV_LAG = 2, 5
HEADS_EARLY = 16
UNROLL = 2


def _layernorm(x, eps=1e-5):
    m = jnp.mean(x, axis=-1, keepdims=True)
    c = x - m
    v = jnp.mean(c * c, axis=-1, keepdims=True)
    return c * lax.rsqrt(v + eps)


def _gelu(x):
    return jax.nn.gelu(x, approximate=True)


def _dot(a, b):
    return jnp.dot(a, b, preferred_element_type=F32)


def _start(copies):
    for cp in copies:
        cp.start()


def _wait(copies):
    for cp in copies:
        cp.wait()


def _weight(ref, slabs=None):
    slabs = range(ref.shape[0]) if slabs is None else slabs
    return jnp.concatenate([pltpu.bitcast(ref.at[c].bitcast(U32)[...], BF16) for c in slabs], axis=1)


def _kernel(x_hbm, mem_hbm, wq_hbm, wk_hbm, wv_hbm, wo_hbm,
            w1_hbm, w2_hbm, w3_hbm, w4_hbm, gw_hbm,
            out_hbm,
            x, mem0, gw, w1, w2, w3, w4, wo, wqkv, stage, hbuf, ybuf, bbuf, gbuf, obuf,
            sems, stage_sems, *, seg, n_heads):
    S, D = x.shape
    M = mem0.shape[0]
    E = LANE
    H = n_heads
    ND = D // LANE

    def copy(src, dst, sem):
        return pltpu.make_async_copy(src, dst, sems.at[sem])

    def slab_copies(src, dst, slabs, sem):
        return [copy(src.at[:, pl.ds(c * LANE, LANE)], dst.at[c], sem) for c in slabs]

    cuts = (0, CUT1 + ROWS, CUT2 + ROWS, S)
    cp_x = [copy(x_hbm.at[pl.ds(lo, hi - lo)], x.at[pl.ds(lo, hi - lo)], k)
            for k, (lo, hi) in enumerate(zip(cuts, cuts[1:]))]
    cp_w1a = slab_copies(w1_hbm, w1, range(W1_FIRST), 3)
    cp_w1b = slab_copies(w1_hbm, w1, range(W1_FIRST, ND), 4)
    cp_w2 = slab_copies(w2_hbm, w2, range(ND), 5)
    cp_w3 = slab_copies(w3_hbm, w3, range(w3.shape[0]), 6)
    cp_w4 = slab_copies(w4_hbm, w4, range(ND), 7)
    cp_wo = slab_copies(wo_hbm, wo, range(ND), 8)
    cp_gw = copy(gw_hbm, gw, 9)
    cp_mem = copy(mem_hbm, mem0, 10)
    out_sem = sems.at[11]

    n3 = S // B3_ROWS
    dch = D // n3
    head_pitch = D // 2 + HEAD_PAD

    def cp_stage(i, slot):
        rows = pl.ds(pl.multiple_of(i * (dch * H), dch * H), dch * H)
        return [pltpu.make_async_copy(w.at[rows], stage.at[slot, t], stage_sems.at[slot, t])
                for t, w in enumerate((wq_hbm, wk_hbm, wv_hbm))]

    def head_row(hd, t):
        return ((t * 2 + hd % 2) * (H // 2) + hd // 2) * head_pitch

    for copies in (cp_x[:1], cp_w1a, cp_w1b, cp_x[1:], cp_w2, cp_w3, cp_w4,
                   [cp_gw, cp_mem], cp_stage(0, 0)):
        _start(copies)
    zeros = jnp.zeros((PAD, LANE), F32)
    for c in range(ND):
        hbuf[c, pl.ds(0, PAD), :] = zeros
        hbuf[c, pl.ds(PAD + S, PAD), :] = zeros

    def normed(r0):
        return _layernorm(x[pl.ds(r0, ROWS), :].astype(F32)).astype(BF16)

    def cache_normed(r0):
        ybuf[pl.ds(r0, ROWS), :] = normed(r0)

    def cached(r0):
        return ybuf[pl.ds(r0, ROWS), :]

    def b1(y, r0, slabs):
        h = _gelu(_dot(y, _weight(w1, slabs)))
        for k, c in enumerate(slabs):
            hbuf[c, pl.ds(PAD + r0, ROWS), :] = h[:, k * LANE:(k + 1) * LANE]

    cp_x[0].wait()
    for r0 in range(0, CUT1, ROWS):
        cache_normed(r0)
    _wait(cp_w1a)
    for r0 in range(0, CUT1, ROWS):
        b1(cached(r0), r0, range(W1_FIRST))
    _wait(cp_w1b)
    for r0 in range(0, CUT1, ROWS):
        b1(cached(r0), r0, range(W1_FIRST, ND))
    cache_normed(CUT1)
    cp_x[1].wait()
    for r0 in range(CUT1, CUT2, ROWS):
        b1(cached(r0) if r0 == CUT1 else normed(r0), r0, range(ND))
    cache_normed(CUT2)
    cp_x[2].wait()
    _wait(cp_w2)
    for r0 in range(CUT2, S, ROWS):
        b1(cached(r0) if r0 == CUT2 else normed(r0), r0, range(ND))

    shifts = (-1, 1, -2, 2)
    for r0 in range(0, S, ROWS):
        g = jnp.concatenate(
            [hbuf[c, pl.ds(PAD + r0 + shifts[c * 4 // ND], ROWS), :].astype(BF16) for c in range(ND)],
            axis=1)
        x1 = x[pl.ds(r0, ROWS), :].astype(F32) + _dot(g, _weight(w2))
        bbuf[pl.ds(r0, ROWS), :] = x1
        ybuf[pl.ds(r0, ROWS), :] = _layernorm(x1).astype(BF16)

    _wait(cp_w3)
    _wait(cp_w4)
    _start(cp_wo)
    cp_gw.wait()
    gw_rows = gw[...].astype(F32)
    gate_w = jnp.concatenate([gw_rows[c:c + 1, :] for c in range(ND)], axis=1)

    def b3_step(i, carry):
        slot = i % 2

        @pl.when(i + 1 < n3)
        def _():
            _start(cp_stage(i + 1, 1 - slot))

        _wait(cp_stage(i, slot))

        for j in range(B3_ROWS // ROWS):
            rows = pl.ds(pl.multiple_of(i * B3_ROWS + j * ROWS, ROWS), ROWS)
            u = _gelu(_dot(ybuf[rows, :], _weight(w3))).astype(BF16)
            b = bbuf[rows, :] + _dot(u, _weight(w4))
            gate = jax.nn.sigmoid(jnp.sum(x[rows, :].astype(F32) * gate_w, axis=-1, keepdims=True))
            bbuf[rows, :] = (1.0 - gate) * b
            gbuf[rows, :] = jnp.broadcast_to(gate, (ROWS, LANE))

        span = (H // 2) * head_pitch + dch // 2
        for t in range(3):
            src = stage.at[slot, t].bitcast(U32)
            dst = [wqkv.at[pl.ds(pl.multiple_of(head_row(hd, t) + i * (dch // 2), 8), span)]
                   for hd in range(2)]
            for r in range(dch // 2):
                for part in range(H // 16):
                    even = src[pl.ds(r * H + part * 8, 8), :]
                    odd = src[pl.ds(r * H + H // 2 + part * 8, 8), :]
                    rows = pl.ds(r + part * 8 * head_pitch, 8, stride=head_pitch)
                    dst[0][rows, :] = (even & LOW16) | (odd << 16)
                    dst[1][rows, :] = (even >> 16) | (odd & HIGH16)
        return carry

    lax.fori_loop(0, n3, b3_step, 0)

    cp_mem.wait()
    _wait(cp_wo)
    scale = E ** -0.5
    row = lax.broadcasted_iota(jnp.int32, (seg + M, seg + M), 0)
    col = lax.broadcasted_iota(jnp.int32, (seg + M, seg + M), 1)
    allow = (row >= seg) | (col >= seg) | (row >= col)

    def head_w(hd, t):
        return pltpu.bitcast(wqkv[pl.ds(head_row(hd, t), D // 2), :], BF16)

    def segment(s, mem):
        rows = pl.ds(pl.multiple_of(s * seg, seg), seg)
        h = jnp.concatenate([x[rows, :].astype(F32), mem], axis=0)
        qk, val, prob, head_out = {}, {}, {}, {}

        def softmax_scores(y):
            sc = lax.dot_general(y[:, :E], y[:, E:], (((1,), (1,)), ((), ())),
                                 preferred_element_type=F32) * scale
            sc = jnp.where(allow, sc, -1e9)
            p = jnp.exp(sc - jnp.max(sc, axis=-1, keepdims=True))
            return p / jnp.sum(p, axis=-1, keepdims=True)

        def out_proj(h0, h1, c):
            o = jnp.concatenate([head_out[hd] for hd in range(h0, h1)], axis=1)
            w = wo.at[c].bitcast(U32)[pl.ds(h0 * E // 2, (h1 - h0) * E // 2), :]
            return _dot(o, pltpu.bitcast(w, BF16))

        early = []
        for t in range(H + ND):
            if t < H:
                qk[t] = _dot(h, jnp.concatenate([head_w(t, 0), head_w(t, 1)], axis=1))
                val[t] = _dot(h, head_w(t, 2))
            else:
                early.append(out_proj(0, HEADS_EARLY, t - H))
            if 0 <= t - QK_LAG < H:
                prob[t - QK_LAG] = softmax_scores(qk.pop(t - QK_LAG))
            if 0 <= t - PV_LAG < H:
                hd = t - PV_LAG
                o = _dot(prob.pop(hd), val.pop(hd))
                head_out[hd] = jnp.concatenate([o[seg:], o[:seg]], axis=0)
        res = jnp.concatenate([out_proj(HEADS_EARLY, H, c) + early[c] for c in range(ND)], axis=1)

        gate = jnp.concatenate([gbuf[rows, :]] * ND, axis=1)
        obuf[rows, :] = (gate * res[M:] + bbuf[rows, :]).astype(obuf.dtype)
        pltpu.make_async_copy(obuf.at[rows], out_hbm.at[rows], out_sem).start()
        return res[:M]

    def a_step(i, mem):
        for u in range(UNROLL):
            mem = segment(i * UNROLL + u, mem)
        return mem

    lax.fori_loop(0, S // seg // UNROLL, a_step, mem0[...].astype(F32))
    pltpu.make_async_copy(obuf, out_hbm, out_sem).wait()


@functools.partial(jax.jit, static_argnames=("A_seg_len",))
def pallas_gated_mix__memory_aug_recurrent_mem_tr__mixer_s_mlp__prompt_kernel(
    A_x: jax.Array,
    A_mem0: jax.Array,
    A_Wq: jax.Array,
    A_Wk: jax.Array,
    A_Wv: jax.Array,
    A_Wo: jax.Array,
    A_seg_len: int,
    B_x: jax.Array,
    B_w1: jax.Array,
    B_w2: jax.Array,
    B_w3: jax.Array,
    B_w4: jax.Array,
    gate_w: jax.Array,
):
    del B_x
    B, S, D = A_x.shape
    M = A_mem0.shape[1]
    _, H, E = A_Wq.shape
    F = B_w3.shape[1]
    seg = int(A_seg_len)
    nd = D // LANE
    dch = D // (S // B3_ROWS)
    assert B == 1 and E == LANE and D % (4 * LANE) == 0 and F % LANE == 0
    assert S % B3_ROWS == 0 and S > CUT2 + ROWS and S % (seg * UNROLL) == 0 and dch % 16 == 0
    assert seg % 16 == 0 and M % 8 == 0 and H % 16 == 0 and HEADS_EARLY + PV_LAG <= H and PV_LAG <= nd

    hbm = pl.BlockSpec(memory_space=pl.ANY)
    out = pl.pallas_call(
        functools.partial(_kernel, seg=seg, n_heads=H),
        out_shape=jax.ShapeDtypeStruct((S, D), A_x.dtype),
        in_specs=[hbm] * 11,
        out_specs=hbm,
        scratch_shapes=[
            pltpu.VMEM((S, D), BF16),
            pltpu.VMEM((M, D), BF16),
            pltpu.VMEM((nd, LANE), BF16),
            pltpu.VMEM((nd, D, LANE), BF16),
            pltpu.VMEM((nd, D, LANE), BF16),
            pltpu.VMEM((F // LANE, D, LANE), BF16),
            pltpu.VMEM((nd, F, LANE), BF16),
            pltpu.VMEM((nd, H * E, LANE), BF16),
            pltpu.VMEM(((3 * H + 8) * (D // 2 + HEAD_PAD), LANE), U32),
            pltpu.VMEM((2, 3, dch * H, LANE), BF16),
            pltpu.VMEM((nd, S + 2 * PAD, LANE), F32),
            pltpu.VMEM((S, D), BF16),
            pltpu.VMEM((S, D), F32),
            pltpu.VMEM((S, LANE), F32),
            pltpu.VMEM((S, D), A_x.dtype),
            pltpu.SemaphoreType.DMA((12,)),
            pltpu.SemaphoreType.DMA((2, 3)),
        ],
        compiler_params=pltpu.CompilerParams(vmem_limit_bytes=112 * 1024 * 1024),
    )(
        A_x.reshape(S, D), A_mem0.reshape(M, D),
        A_Wq.reshape(D * H, E), A_Wk.reshape(D * H, E), A_Wv.reshape(D * H, E),
        A_Wo.reshape(H * E, D),
        B_w1, B_w2, B_w3, B_w4, gate_w.reshape(nd, LANE),
    )
    return out.reshape(B, S, D)
```

```python
import functools

import jax
import jax.numpy as jnp
import numpy as np
from jax import lax
import jax.experimental.pallas as pl
import jax.experimental.pallas.tpu as pltpu

F32, BF16, U32 = jnp.float32, jnp.bfloat16, jnp.uint32
LOW16, HIGH16 = np.uint32(0xFFFF), np.uint32(0xFFFF0000)
LANE = 128
PAD = 8
HEAD_PAD = 4

ROWS = 64
CUT1, CUT2 = 384, 832
W1_STEP = 2
B3_ROWS = 256
QK_LAG, PV_LAG = 2, 5
HEADS_EARLY = 16
UNROLL = 3


def _layernorm(x, eps=1e-5):
    m = jnp.mean(x, axis=-1, keepdims=True)
    c = x - m
    v = jnp.mean(c * c, axis=-1, keepdims=True)
    return c * lax.rsqrt(v + eps)


def _gelu(x):
    return jax.nn.gelu(x, approximate=True)


def _dot(a, b):
    return jnp.dot(a, b, preferred_element_type=F32)


def _start(copies):
    for cp in copies:
        cp.start()


def _wait(copies):
    for cp in copies:
        cp.wait()


def _weight(ref, slabs=None):
    slabs = range(ref.shape[0]) if slabs is None else slabs
    return jnp.concatenate([pltpu.bitcast(ref.at[c].bitcast(U32)[...], BF16) for c in slabs], axis=1)


def _kernel(x_hbm, mem_hbm, wq_hbm, wk_hbm, wv_hbm, wo_hbm,
            w1_hbm, w2_hbm, w3_hbm, w4_hbm, gw_hbm,
            out_hbm,
            x, mem0, gw, w1, w2, w3, w4, wo, wqkv, stage, hbuf, ybuf, bbuf, gbuf, obuf,
            sems, stage_sems, *, seg, n_heads):
    S, D = x.shape
    M = mem0.shape[0]
    E = LANE
    H = n_heads
    ND = D // LANE

    def copy(src, dst, sem):
        return pltpu.make_async_copy(src, dst, sems.at[sem])

    def slab_copies(src, dst, slabs, sem):
        return [copy(src.at[:, pl.ds(c * LANE, LANE)], dst.at[c], sem) for c in slabs]

    cuts = (0, CUT1 + ROWS, CUT2 + ROWS, S)
    cp_x = [copy(x_hbm.at[pl.ds(lo, hi - lo)], x.at[pl.ds(lo, hi - lo)], k)
            for k, (lo, hi) in enumerate(zip(cuts, cuts[1:]))]
    cp_w2 = slab_copies(w2_hbm, w2, range(ND), 3)
    cp_w3 = slab_copies(w3_hbm, w3, range(w3.shape[0]), 4)
    cp_w4 = slab_copies(w4_hbm, w4, range(ND), 5)
    cp_wo = slab_copies(wo_hbm, wo, range(ND), 6)
    cp_gw = copy(gw_hbm, gw, 7)
    cp_mem = copy(mem_hbm, mem0, 8)
    out_sem = sems.at[9]
    w1_groups = [range(c, min(c + W1_STEP, ND)) for c in range(0, ND, W1_STEP)]
    cp_w1 = [slab_copies(w1_hbm, w1, slabs, 10 + k) for k, slabs in enumerate(w1_groups)]

    n3 = S // B3_ROWS
    dch = D // n3
    head_pitch = D // 2 + HEAD_PAD

    def cp_stage(i, slot):
        rows = pl.ds(pl.multiple_of(i * (dch * H), dch * H), dch * H)
        return [pltpu.make_async_copy(w.at[rows], stage.at[slot, t], stage_sems.at[slot, t])
                for t, w in enumerate((wq_hbm, wk_hbm, wv_hbm))]

    def head_row(hd, t):
        return ((t * 2 + hd % 2) * (H // 2) + hd // 2) * head_pitch

    for copies in (cp_x[:1], *cp_w1, cp_x[1:], cp_w2, cp_w3, cp_w4,
                   [cp_gw, cp_mem], cp_stage(0, 0)):
        _start(copies)
    zeros = jnp.zeros((PAD, LANE), F32)
    for c in range(ND):
        hbuf[c, pl.ds(0, PAD), :] = zeros
        hbuf[c, pl.ds(PAD + S, PAD), :] = zeros

    def normed(r0):
        return _layernorm(x[pl.ds(r0, ROWS), :].astype(F32)).astype(BF16)

    def cache_normed(r0):
        ybuf[pl.ds(r0, ROWS), :] = normed(r0)

    def cached(r0):
        return ybuf[pl.ds(r0, ROWS), :]

    def b1(y, r0, slabs):
        h = _gelu(_dot(y, _weight(w1, slabs)))
        for k, c in enumerate(slabs):
            hbuf[c, pl.ds(PAD + r0, ROWS), :] = h[:, k * LANE:(k + 1) * LANE]

    cp_x[0].wait()
    for r0 in range(0, CUT1, ROWS):
        cache_normed(r0)
    for slabs, copies in zip(w1_groups, cp_w1):
        _wait(copies)
        for r0 in range(0, CUT1, ROWS):
            b1(cached(r0), r0, slabs)
    cache_normed(CUT1)
    cp_x[1].wait()
    for r0 in range(CUT1, CUT2, ROWS):
        b1(cached(r0) if r0 == CUT1 else normed(r0), r0, range(ND))
    cache_normed(CUT2)
    cp_x[2].wait()
    for r0 in range(CUT2, S, ROWS):
        b1(cached(r0) if r0 == CUT2 else normed(r0), r0, range(ND))

    _wait(cp_w2)
    shifts = (-1, 1, -2, 2)
    for r0 in range(0, S, ROWS):
        g = jnp.concatenate(
            [hbuf[c, pl.ds(PAD + r0 + shifts[c * 4 // ND], ROWS), :].astype(BF16) for c in range(ND)],
            axis=1)
        x1 = x[pl.ds(r0, ROWS), :].astype(F32) + _dot(g, _weight(w2))
        bbuf[pl.ds(r0, ROWS), :] = x1
        ybuf[pl.ds(r0, ROWS), :] = _layernorm(x1).astype(BF16)

    _wait(cp_w3)
    _wait(cp_w4)
    _start(cp_wo)
    cp_gw.wait()
    gw_rows = gw[...].astype(F32)
    gate_w = jnp.concatenate([gw_rows[c:c + 1, :] for c in range(ND)], axis=1)

    def b3_step(i, carry):
        slot = i % 2

        @pl.when(i + 1 < n3)
        def _():
            _start(cp_stage(i + 1, 1 - slot))

        _wait(cp_stage(i, slot))

        for j in range(B3_ROWS // ROWS):
            rows = pl.ds(pl.multiple_of(i * B3_ROWS + j * ROWS, ROWS), ROWS)
            u = _gelu(_dot(ybuf[rows, :], _weight(w3))).astype(BF16)
            b = bbuf[rows, :] + _dot(u, _weight(w4))
            gate = jax.nn.sigmoid(jnp.sum(x[rows, :].astype(F32) * gate_w, axis=-1, keepdims=True))
            bbuf[rows, :] = (1.0 - gate) * b
            gbuf[rows, :] = jnp.broadcast_to(gate, (ROWS, LANE))

        span = (H // 2) * head_pitch + dch // 2
        for t in range(3):
            src = stage.at[slot, t].bitcast(U32)
            dst = [wqkv.at[pl.ds(pl.multiple_of(head_row(hd, t) + i * (dch // 2), 8), span)]
                   for hd in range(2)]
            for r in range(dch // 2):
                for part in range(H // 16):
                    even = src[pl.ds(r * H + part * 8, 8), :]
                    odd = src[pl.ds(r * H + H // 2 + part * 8, 8), :]
                    rows = pl.ds(r + part * 8 * head_pitch, 8, stride=head_pitch)
                    dst[0][rows, :] = (even & LOW16) | (odd << 16)
                    dst[1][rows, :] = (even >> 16) | (odd & HIGH16)
        return carry

    lax.fori_loop(0, n3, b3_step, 0)

    cp_mem.wait()
    _wait(cp_wo)
    scale = E ** -0.5
    row = lax.broadcasted_iota(jnp.int32, (seg + M, seg + M), 0)
    col = lax.broadcasted_iota(jnp.int32, (seg + M, seg + M), 1)
    allow = (row >= seg) | (col >= seg) | (row >= col)

    def head_w(hd, t):
        return pltpu.bitcast(wqkv[pl.ds(head_row(hd, t), D // 2), :], BF16)

    def segment(s, mem):
        r0 = s * seg
        rows = pl.ds(r0 if isinstance(r0, int) else pl.multiple_of(r0, seg), seg)
        h = jnp.concatenate([x[rows, :].astype(F32), mem], axis=0)
        qk, val, prob, head_out = {}, {}, {}, {}

        def softmax_scores(y):
            sc = lax.dot_general(y[:, :E], y[:, E:], (((1,), (1,)), ((), ())),
                                 preferred_element_type=F32) * scale
            sc = jnp.where(allow, sc, -1e9)
            p = jnp.exp(sc - jnp.max(sc, axis=-1, keepdims=True))
            return p / jnp.sum(p, axis=-1, keepdims=True)

        def out_proj(h0, h1, c):
            o = jnp.concatenate([head_out[hd] for hd in range(h0, h1)], axis=1)
            w = wo.at[c].bitcast(U32)[pl.ds(h0 * E // 2, (h1 - h0) * E // 2), :]
            return _dot(o, pltpu.bitcast(w, BF16))

        early = []
        for t in range(H + ND):
            if t < H:
                qk[t] = _dot(h, jnp.concatenate([head_w(t, 0), head_w(t, 1)], axis=1))
                val[t] = _dot(h, head_w(t, 2))
            else:
                early.append(out_proj(0, HEADS_EARLY, t - H))
            if 0 <= t - QK_LAG < H:
                prob[t - QK_LAG] = softmax_scores(qk.pop(t - QK_LAG))
            if 0 <= t - PV_LAG < H:
                hd = t - PV_LAG
                o = _dot(prob.pop(hd), val.pop(hd))
                head_out[hd] = jnp.concatenate([o[seg:], o[:seg]], axis=0)
        res = jnp.concatenate([out_proj(HEADS_EARLY, H, c) + early[c] for c in range(ND)], axis=1)

        gate = jnp.concatenate([gbuf[rows, :]] * ND, axis=1)
        obuf[rows, :] = (gate * res[M:] + bbuf[rows, :]).astype(obuf.dtype)
        pltpu.make_async_copy(obuf.at[rows], out_hbm.at[rows], out_sem).start()
        return res[:M]

    def a_step(i, mem):
        for u in range(UNROLL):
            mem = segment(i * UNROLL + u, mem)
        return mem

    n_seg = S // seg
    mem = lax.fori_loop(0, n_seg // UNROLL, a_step, mem0[...].astype(F32))
    for s in range(n_seg - n_seg % UNROLL, n_seg):
        mem = segment(s, mem)
    pltpu.make_async_copy(obuf, out_hbm, out_sem).wait()


@functools.partial(jax.jit, static_argnames=("A_seg_len",))
def pallas_gated_mix__memory_aug_recurrent_mem_tr__mixer_s_mlp__prompt_kernel(
    A_x: jax.Array,
    A_mem0: jax.Array,
    A_Wq: jax.Array,
    A_Wk: jax.Array,
    A_Wv: jax.Array,
    A_Wo: jax.Array,
    A_seg_len: int,
    B_x: jax.Array,
    B_w1: jax.Array,
    B_w2: jax.Array,
    B_w3: jax.Array,
    B_w4: jax.Array,
    gate_w: jax.Array,
):
    del B_x
    B, S, D = A_x.shape
    M = A_mem0.shape[1]
    _, H, E = A_Wq.shape
    F = B_w3.shape[1]
    seg = int(A_seg_len)
    nd = D // LANE
    dch = D // (S // B3_ROWS)
    assert B == 1 and E == LANE and D % (4 * LANE) == 0 and F % LANE == 0
    assert S % B3_ROWS == 0 and S > CUT2 + ROWS and S % seg == 0 and dch % 16 == 0
    assert seg % 16 == 0 and M % 8 == 0 and H % 16 == 0 and HEADS_EARLY + PV_LAG <= H and PV_LAG <= nd

    hbm = pl.BlockSpec(memory_space=pl.ANY)
    out = pl.pallas_call(
        functools.partial(_kernel, seg=seg, n_heads=H),
        out_shape=jax.ShapeDtypeStruct((S, D), A_x.dtype),
        in_specs=[hbm] * 11,
        out_specs=hbm,
        scratch_shapes=[
            pltpu.VMEM((S, D), BF16),
            pltpu.VMEM((M, D), BF16),
            pltpu.VMEM((nd, LANE), BF16),
            pltpu.VMEM((nd, D, LANE), BF16),
            pltpu.VMEM((nd, D, LANE), BF16),
            pltpu.VMEM((F // LANE, D, LANE), BF16),
            pltpu.VMEM((nd, F, LANE), BF16),
            pltpu.VMEM((nd, H * E, LANE), BF16),
            pltpu.VMEM(((3 * H + 8) * (D // 2 + HEAD_PAD), LANE), U32),
            pltpu.VMEM((2, 3, dch * H, LANE), BF16),
            pltpu.VMEM((nd, S + 2 * PAD, LANE), F32),
            pltpu.VMEM((S, D), BF16),
            pltpu.VMEM((S, D), F32),
            pltpu.VMEM((S, LANE), F32),
            pltpu.VMEM((S, D), A_x.dtype),
            pltpu.SemaphoreType.DMA((10 + nd,)),
            pltpu.SemaphoreType.DMA((2, 3)),
        ],
        compiler_params=pltpu.CompilerParams(vmem_limit_bytes=112 * 1024 * 1024),
    )(
        A_x.reshape(S, D), A_mem0.reshape(M, D),
        A_Wq.reshape(D * H, E), A_Wk.reshape(D * H, E), A_Wv.reshape(D * H, E),
        A_Wo.reshape(H * E, D),
        B_w1, B_w2, B_w3, B_w4, gate_w.reshape(nd, LANE),
    )
    return out.reshape(B, S, D)
```

```python
import functools

import jax
import jax.numpy as jnp
import numpy as np
from jax import lax
import jax.experimental.pallas as pl
import jax.experimental.pallas.tpu as pltpu

F32, BF16, U32 = jnp.float32, jnp.bfloat16, jnp.uint32
LOW16, HIGH16 = np.uint32(0xFFFF), np.uint32(0xFFFF0000)
LANE = 128
PAD = 8
HEAD_PAD = 4

ROWS = 64
CUT1, CUT2 = 384, 832
W1_STEP = 2
B3_ROWS = 256
QK_LAG, PV_LAG = 2, 5
HEADS_EARLY = 16
UNROLL = 3


def _layernorm(x, eps=1e-5):
    m = jnp.mean(x, axis=-1, keepdims=True)
    c = x - m
    v = jnp.mean(c * c, axis=-1, keepdims=True)
    return c * lax.rsqrt(v + eps)


def _gelu(x):
    return jax.nn.gelu(x, approximate=True)


def _dot(a, b):
    return jnp.dot(a, b, preferred_element_type=F32)


def _start(copies):
    for cp in copies:
        cp.start()


def _wait(copies):
    for cp in copies:
        cp.wait()


def _weight(ref, slabs=None):
    slabs = range(ref.shape[0]) if slabs is None else slabs
    return jnp.concatenate([pltpu.bitcast(ref.at[c].bitcast(U32)[...], BF16) for c in slabs], axis=1)


def _kernel(x_hbm, mem_hbm, wq_hbm, wk_hbm, wv_hbm, wo_hbm,
            w1_hbm, w2_hbm, w3_hbm, w4_hbm, gw_hbm,
            out_hbm,
            x, mem0, gw, w1, w2, w3, w4, wo, wqkv, stage, hbuf, ybuf, bbuf, gbuf, obuf,
            sems, stage_sems, *, seg, n_heads):
    S, D = x.shape
    M = mem0.shape[0]
    E = LANE
    H = n_heads
    ND = D // LANE

    def copy(src, dst, sem):
        return pltpu.make_async_copy(src, dst, sems.at[sem])

    def slab_copies(src, dst, slabs, sem):
        return [copy(src.at[:, pl.ds(c * LANE, LANE)], dst.at[c], sem) for c in slabs]

    cuts = (0, CUT1 + ROWS, CUT2 + ROWS, S)
    cp_x = [copy(x_hbm.at[pl.ds(lo, hi - lo)], x.at[pl.ds(lo, hi - lo)], k)
            for k, (lo, hi) in enumerate(zip(cuts, cuts[1:]))]
    cp_w2 = slab_copies(w2_hbm, w2, range(ND), 3)
    cp_w3 = slab_copies(w3_hbm, w3, range(w3.shape[0]), 4)
    cp_w4 = slab_copies(w4_hbm, w4, range(ND), 5)
    cp_wo = slab_copies(wo_hbm, wo, range(ND), 6)
    cp_gw = copy(gw_hbm, gw, 7)
    cp_mem = copy(mem_hbm, mem0, 8)
    out_sem = sems.at[9]
    w1_groups = [range(c, min(c + W1_STEP, ND)) for c in range(0, ND, W1_STEP)]
    cp_w1 = [slab_copies(w1_hbm, w1, slabs, 10 + k) for k, slabs in enumerate(w1_groups)]

    n3 = S // B3_ROWS
    dch = D // n3
    head_pitch = D // 2 + HEAD_PAD

    def cp_stage(i, slot):
        rows = pl.ds(pl.multiple_of(i * (dch * H), dch * H), dch * H)
        return [pltpu.make_async_copy(w.at[rows], stage.at[slot, t], stage_sems.at[slot, t])
                for t, w in enumerate((wq_hbm, wk_hbm, wv_hbm))]

    def head_row(hd, t):
        return ((t * 2 + hd % 2) * (H // 2) + hd // 2) * head_pitch

    for copies in (cp_x[:1], *cp_w1, cp_x[1:], cp_w2, cp_w3, cp_w4,
                   [cp_gw, cp_mem], cp_stage(0, 0)):
        _start(copies)
    zeros = jnp.zeros((PAD, LANE), F32)
    for c in range(ND):
        hbuf[c, pl.ds(0, PAD), :] = zeros
        hbuf[c, pl.ds(PAD + S, PAD), :] = zeros

    def normed(r0):
        return _layernorm(x[pl.ds(r0, ROWS), :].astype(F32)).astype(BF16)

    def cache_normed(r0):
        ybuf[pl.ds(r0, ROWS), :] = normed(r0)

    def cached(r0):
        return ybuf[pl.ds(r0, ROWS), :]

    def b1(y, r0, slabs):
        h = _gelu(_dot(y, _weight(w1, slabs)))
        for k, c in enumerate(slabs):
            hbuf[c, pl.ds(PAD + r0, ROWS), :] = h[:, k * LANE:(k + 1) * LANE]

    cp_x[0].wait()
    for r0 in range(0, CUT1, ROWS):
        cache_normed(r0)
    for slabs, copies in zip(w1_groups, cp_w1):
        _wait(copies)
        for r0 in range(0, CUT1, ROWS):
            b1(cached(r0), r0, slabs)
    cache_normed(CUT1)
    cp_x[1].wait()
    for r0 in range(CUT1, CUT2, ROWS):
        b1(cached(r0) if r0 == CUT1 else normed(r0), r0, range(ND))
    cache_normed(CUT2)
    cp_x[2].wait()
    for r0 in range(CUT2, S, ROWS):
        b1(cached(r0) if r0 == CUT2 else normed(r0), r0, range(ND))

    _wait(cp_w2)
    shifts = (-1, 1, -2, 2)
    for r0 in range(0, S, ROWS):
        g = jnp.concatenate(
            [hbuf[c, pl.ds(PAD + r0 + shifts[c * 4 // ND], ROWS), :].astype(BF16) for c in range(ND)],
            axis=1)
        x1 = x[pl.ds(r0, ROWS), :].astype(F32) + _dot(g, _weight(w2))
        bbuf[pl.ds(r0, ROWS), :] = x1
        ybuf[pl.ds(r0, ROWS), :] = _layernorm(x1).astype(BF16)

    _wait(cp_w3)
    _wait(cp_w4)
    _start(cp_wo)
    cp_gw.wait()
    gw_rows = gw[...].astype(F32)
    gate_w = jnp.concatenate([gw_rows[c:c + 1, :] for c in range(ND)], axis=1)

    def b3_step(i, carry):
        slot = i % 2

        @pl.when(i + 1 < n3)
        def _():
            _start(cp_stage(i + 1, 1 - slot))

        _wait(cp_stage(i, slot))

        for j in range(B3_ROWS // ROWS):
            rows = pl.ds(pl.multiple_of(i * B3_ROWS + j * ROWS, ROWS), ROWS)
            u = _gelu(_dot(ybuf[rows, :], _weight(w3))).astype(BF16)
            b = bbuf[rows, :] + _dot(u, _weight(w4))
            gate = jax.nn.sigmoid(jnp.sum(x[rows, :].astype(F32) * gate_w, axis=-1, keepdims=True))
            bbuf[rows, :] = (1.0 - gate) * b
            gbuf[rows, :] = jnp.broadcast_to(gate, (ROWS, LANE))

        span = (H // 2) * head_pitch + dch // 2
        for t in range(3):
            src = stage.at[slot, t].bitcast(U32)
            dst = [wqkv.at[pl.ds(pl.multiple_of(head_row(hd, t) + i * (dch // 2), 8), span)]
                   for hd in range(2)]
            for r in range(dch // 2):
                for part in range(H // 16):
                    even = src[pl.ds(r * H + part * 8, 8), :]
                    odd = src[pl.ds(r * H + H // 2 + part * 8, 8), :]
                    rows = pl.ds(r + part * 8 * head_pitch, 8, stride=head_pitch)
                    dst[0][rows, :] = (even & LOW16) | (odd << 16)
                    dst[1][rows, :] = (even >> 16) | (odd & HIGH16)
        return carry

    lax.fori_loop(0, n3, b3_step, 0)

    cp_mem.wait()
    _wait(cp_wo)
    scale = E ** -0.5
    row = lax.broadcasted_iota(jnp.int32, (seg + M, seg + M), 0)
    col = lax.broadcasted_iota(jnp.int32, (seg + M, seg + M), 1)
    allow = (row >= seg) | (col >= seg) | (row >= col)

    def head_w(hd, t):
        return pltpu.bitcast(wqkv[pl.ds(head_row(hd, t), D // 2), :], BF16)

    def segment(s, mem):
        r0 = s * seg
        rows = pl.ds(r0 if isinstance(r0, int) else pl.multiple_of(r0, seg), seg)
        h = jnp.concatenate([x[rows, :].astype(F32), mem], axis=0)
        qk, val, prob, head_out = {}, {}, {}, {}

        def softmax_scores(y):
            sc = lax.dot_general(y[:, :E], y[:, E:], (((1,), (1,)), ((), ())),
                                 preferred_element_type=F32) * scale
            sc = jnp.where(allow, sc, -1e9)
            p = jnp.exp(sc - jnp.max(sc, axis=-1, keepdims=True))
            return p / jnp.sum(p, axis=-1, keepdims=True)

        def out_proj(h0, h1, c):
            o = jnp.concatenate([head_out[hd] for hd in range(h0, h1)], axis=1)
            w = wo.at[c].bitcast(U32)[pl.ds(h0 * E // 2, (h1 - h0) * E // 2), :]
            return _dot(o, pltpu.bitcast(w, BF16))

        early = []
        for t in range(H + ND):
            if t == 0:
                w = jnp.concatenate([head_w(0, k) for k in range(3)], axis=1)
                first = _dot(h[:, :D // 2], w[:D // 2])
                y = _dot(h[:, D // 2:], w[D // 2:]) + first
                qk[0], val[0] = y[:, :2 * E], y[:, 2 * E:]
            elif t < H:
                qk[t] = _dot(h, jnp.concatenate([head_w(t, 0), head_w(t, 1)], axis=1))
                val[t] = _dot(h, head_w(t, 2))
            else:
                early.append(out_proj(0, HEADS_EARLY, t - H))
            if 0 <= t - QK_LAG < H:
                prob[t - QK_LAG] = softmax_scores(qk.pop(t - QK_LAG))
            if 0 <= t - PV_LAG < H:
                hd = t - PV_LAG
                o = _dot(prob.pop(hd), val.pop(hd))
                head_out[hd] = jnp.concatenate([o[seg:], o[:seg]], axis=0)
        res = jnp.concatenate([out_proj(HEADS_EARLY, H, c) + early[c] for c in range(ND)], axis=1)

        gate = jnp.concatenate([gbuf[rows, :]] * ND, axis=1)
        obuf[rows, :] = (gate * res[M:] + bbuf[rows, :]).astype(obuf.dtype)
        pltpu.make_async_copy(obuf.at[rows], out_hbm.at[rows], out_sem).start()
        return res[:M]

    def a_step(i, mem):
        for u in range(UNROLL):
            mem = segment(i * UNROLL + u, mem)
        return mem

    n_seg = S // seg
    mem = lax.fori_loop(0, n_seg // UNROLL, a_step, mem0[...].astype(F32))
    for s in range(n_seg - n_seg % UNROLL, n_seg):
        mem = segment(s, mem)
    pltpu.make_async_copy(obuf, out_hbm, out_sem).wait()


@functools.partial(jax.jit, static_argnames=("A_seg_len",))
def pallas_gated_mix__memory_aug_recurrent_mem_tr__mixer_s_mlp__prompt_kernel(
    A_x: jax.Array,
    A_mem0: jax.Array,
    A_Wq: jax.Array,
    A_Wk: jax.Array,
    A_Wv: jax.Array,
    A_Wo: jax.Array,
    A_seg_len: int,
    B_x: jax.Array,
    B_w1: jax.Array,
    B_w2: jax.Array,
    B_w3: jax.Array,
    B_w4: jax.Array,
    gate_w: jax.Array,
):
    del B_x
    B, S, D = A_x.shape
    M = A_mem0.shape[1]
    _, H, E = A_Wq.shape
    F = B_w3.shape[1]
    seg = int(A_seg_len)
    nd = D // LANE
    dch = D // (S // B3_ROWS)
    assert B == 1 and E == LANE and D % (4 * LANE) == 0 and F % LANE == 0
    assert S % B3_ROWS == 0 and S > CUT2 + ROWS and S % seg == 0 and dch % 16 == 0
    assert seg % 16 == 0 and M % 8 == 0 and H % 16 == 0 and HEADS_EARLY + PV_LAG <= H and PV_LAG <= nd

    hbm = pl.BlockSpec(memory_space=pl.ANY)
    out = pl.pallas_call(
        functools.partial(_kernel, seg=seg, n_heads=H),
        out_shape=jax.ShapeDtypeStruct((S, D), A_x.dtype),
        in_specs=[hbm] * 11,
        out_specs=hbm,
        scratch_shapes=[
            pltpu.VMEM((S, D), BF16),
            pltpu.VMEM((M, D), BF16),
            pltpu.VMEM((nd, LANE), BF16),
            pltpu.VMEM((nd, D, LANE), BF16),
            pltpu.VMEM((nd, D, LANE), BF16),
            pltpu.VMEM((F // LANE, D, LANE), BF16),
            pltpu.VMEM((nd, F, LANE), BF16),
            pltpu.VMEM((nd, H * E, LANE), BF16),
            pltpu.VMEM(((3 * H + 8) * (D // 2 + HEAD_PAD), LANE), U32),
            pltpu.VMEM((2, 3, dch * H, LANE), BF16),
            pltpu.VMEM((nd, S + 2 * PAD, LANE), F32),
            pltpu.VMEM((S, D), BF16),
            pltpu.VMEM((S, D), F32),
            pltpu.VMEM((S, LANE), F32),
            pltpu.VMEM((S, D), A_x.dtype),
            pltpu.SemaphoreType.DMA((10 + nd,)),
            pltpu.SemaphoreType.DMA((2, 3)),
        ],
        compiler_params=pltpu.CompilerParams(vmem_limit_bytes=112 * 1024 * 1024),
    )(
        A_x.reshape(S, D), A_mem0.reshape(M, D),
        A_Wq.reshape(D * H, E), A_Wk.reshape(D * H, E), A_Wv.reshape(D * H, E),
        A_Wo.reshape(H * E, D),
        B_w1, B_w2, B_w3, B_w4, gate_w.reshape(nd, LANE),
    )
    return out.reshape(B, S, D)
```

```python
import functools

import jax
import jax.numpy as jnp
import numpy as np
from jax import lax
import jax.experimental.pallas as pl
import jax.experimental.pallas.tpu as pltpu

F32, BF16, U32 = jnp.float32, jnp.bfloat16, jnp.uint32
LOW16, HIGH16 = np.uint32(0xFFFF), np.uint32(0xFFFF0000)
LANE = 128
PAD = 8
HEAD_PAD = 4

ROWS = 64
CUT1, CUT2 = 384, 832
W1_STEP = 2
B3_ROWS = 256
QK_LAG, PV_LAG = 2, 5
HEADS_EARLY = 16
UNROLL = 3


def _layernorm(x, eps=1e-5):
    m = jnp.mean(x, axis=-1, keepdims=True)
    c = x - m
    v = jnp.mean(c * c, axis=-1, keepdims=True)
    return c * lax.rsqrt(v + eps)


def _gelu(x):
    return jax.nn.gelu(x, approximate=True)


def _dot(a, b):
    return jnp.dot(a, b, preferred_element_type=F32)


def _start(copies):
    for cp in copies:
        cp.start()


def _wait(copies):
    for cp in copies:
        cp.wait()


def _weight(ref, slabs=None):
    slabs = range(ref.shape[0]) if slabs is None else slabs
    return jnp.concatenate([pltpu.bitcast(ref.at[c].bitcast(U32)[...], BF16) for c in slabs], axis=1)


def _kernel(x_hbm, mem_hbm, wq_hbm, wk_hbm, wv_hbm, wo_hbm,
            w1_hbm, w2_hbm, w3_hbm, w4_hbm, gw_hbm,
            out_hbm,
            x, mem0, gw, w1, w2, w3, w4, wo, wqkv, stage, hbuf, ybuf, bbuf, gbuf, obuf,
            sems, stage_sems, *, seg, n_heads):
    S, D = x.shape
    M = mem0.shape[0]
    E = LANE
    H = n_heads
    ND = D // LANE

    def copy(src, dst, sem):
        return pltpu.make_async_copy(src, dst, sems.at[sem])

    def slab_copies(src, dst, slabs, sem):
        return [copy(src.at[:, pl.ds(c * LANE, LANE)], dst.at[c], sem) for c in slabs]

    cuts = (0, CUT1 + ROWS, CUT2 + ROWS, S)
    cp_x = [copy(x_hbm.at[pl.ds(lo, hi - lo)], x.at[pl.ds(lo, hi - lo)], k)
            for k, (lo, hi) in enumerate(zip(cuts, cuts[1:]))]
    cp_w2 = slab_copies(w2_hbm, w2, range(ND), 3)
    cp_w3 = slab_copies(w3_hbm, w3, range(w3.shape[0]), 4)
    cp_w4 = slab_copies(w4_hbm, w4, range(ND), 5)
    cp_wo = slab_copies(wo_hbm, wo, range(ND), 6)
    cp_gw = copy(gw_hbm, gw, 7)
    cp_mem = copy(mem_hbm, mem0, 8)
    out_sem = sems.at[9]
    w1_groups = [range(c, min(c + W1_STEP, ND)) for c in range(0, ND, W1_STEP)]
    cp_w1 = [slab_copies(w1_hbm, w1, slabs, 10 + k) for k, slabs in enumerate(w1_groups)]

    n3 = S // B3_ROWS
    dch = D // n3
    head_pitch = D // 2 + HEAD_PAD

    def cp_stage(i, slot):
        rows = pl.ds(pl.multiple_of(i * (dch * H), dch * H), dch * H)
        return [pltpu.make_async_copy(w.at[rows], stage.at[slot, t], stage_sems.at[slot, t])
                for t, w in enumerate((wq_hbm, wk_hbm, wv_hbm))]

    def head_row(hd, t):
        return ((t * 2 + hd % 2) * (H // 2) + hd // 2) * head_pitch

    for copies in (cp_x[:1], *cp_w1, cp_x[1:], cp_w2, cp_w3, cp_w4,
                   [cp_gw, cp_mem], cp_stage(0, 0)):
        _start(copies)
    zeros = jnp.zeros((PAD, LANE), F32)
    for c in range(ND):
        hbuf[c, pl.ds(0, PAD), :] = zeros
        hbuf[c, pl.ds(PAD + S, PAD), :] = zeros

    def normed(r0):
        return _layernorm(x[pl.ds(r0, ROWS), :].astype(F32)).astype(BF16)

    def cache_normed(r0):
        ybuf[pl.ds(r0, ROWS), :] = normed(r0)

    def cached(r0):
        return ybuf[pl.ds(r0, ROWS), :]

    def b1(y, r0, slabs):
        h = _gelu(_dot(y, _weight(w1, slabs)))
        for k, c in enumerate(slabs):
            hbuf[c, pl.ds(PAD + r0, ROWS), :] = h[:, k * LANE:(k + 1) * LANE]

    cp_x[0].wait()
    for r0 in range(0, CUT1, ROWS):
        cache_normed(r0)
    for slabs, copies in zip(w1_groups, cp_w1):
        _wait(copies)
        for r0 in range(0, CUT1, ROWS):
            b1(cached(r0), r0, slabs)
    cache_normed(CUT1)
    cp_x[1].wait()
    for r0 in range(CUT1, CUT2, ROWS):
        b1(cached(r0) if r0 == CUT1 else normed(r0), r0, range(ND))
    cache_normed(CUT2)
    cp_x[2].wait()
    for r0 in range(CUT2, S, ROWS):
        b1(cached(r0) if r0 == CUT2 else normed(r0), r0, range(ND))

    _wait(cp_w2)
    shifts = (-1, 1, -2, 2)
    for r0 in range(0, S, ROWS):
        g = jnp.concatenate(
            [hbuf[c, pl.ds(PAD + r0 + shifts[c * 4 // ND], ROWS), :].astype(BF16) for c in range(ND)],
            axis=1)
        x1 = x[pl.ds(r0, ROWS), :].astype(F32) + _dot(g, _weight(w2))
        bbuf[pl.ds(r0, ROWS), :] = x1
        ybuf[pl.ds(r0, ROWS), :] = _layernorm(x1).astype(BF16)

    _wait(cp_w3)
    _wait(cp_w4)
    _start(cp_wo)
    cp_gw.wait()
    gw_rows = gw[...].astype(F32)
    gate_w = jnp.concatenate([gw_rows[c:c + 1, :] for c in range(ND)], axis=1)

    def b3_step(i, carry):
        slot = i % 2

        @pl.when(i + 1 < n3)
        def _():
            _start(cp_stage(i + 1, 1 - slot))

        _wait(cp_stage(i, slot))

        for j in range(B3_ROWS // ROWS):
            rows = pl.ds(pl.multiple_of(i * B3_ROWS + j * ROWS, ROWS), ROWS)
            u = _gelu(_dot(ybuf[rows, :], _weight(w3))).astype(BF16)
            b = bbuf[rows, :] + _dot(u, _weight(w4))
            gate = jax.nn.sigmoid(jnp.sum(x[rows, :].astype(F32) * gate_w, axis=-1, keepdims=True))
            bbuf[rows, :] = (1.0 - gate) * b
            gbuf[rows, :] = jnp.broadcast_to(gate, (ROWS, LANE))

        span = (H // 2) * head_pitch + dch // 2
        for t in range(3):
            src = stage.at[slot, t].bitcast(U32)
            dst = [wqkv.at[pl.ds(pl.multiple_of(head_row(hd, t) + i * (dch // 2), 8), span)]
                   for hd in range(2)]
            for r in range(dch // 2):
                for part in range(H // 16):
                    even = src[pl.ds(r * H + part * 8, 8), :]
                    odd = src[pl.ds(r * H + H // 2 + part * 8, 8), :]
                    rows = pl.ds(r + part * 8 * head_pitch, 8, stride=head_pitch)
                    dst[0][rows, :] = (even & LOW16) | (odd << 16)
                    dst[1][rows, :] = (even >> 16) | (odd & HIGH16)
        return carry

    lax.fori_loop(0, n3, b3_step, 0)

    cp_mem.wait()
    _wait(cp_wo)
    scale = E ** -0.5
    row = lax.broadcasted_iota(jnp.int32, (seg + M, seg + M), 0)
    col = lax.broadcasted_iota(jnp.int32, (seg + M, seg + M), 1)
    allow = (row >= seg) | (col >= seg) | (row >= col)

    def head_w(hd, t):
        return pltpu.bitcast(wqkv[pl.ds(head_row(hd, t), D // 2), :], BF16)

    def segment(s, mem, last=False):
        r0 = s * seg
        rows = pl.ds(r0 if isinstance(r0, int) else pl.multiple_of(r0, seg), seg)
        h = jnp.concatenate([x[rows, :].astype(F32), mem], axis=0)
        n_mem = 0 if last else M
        query, key, val, prob, head_out = {}, {}, {}, {}, {}

        def project(hd):
            if hd == 0:
                w = jnp.concatenate([head_w(hd, t) for t in range(3)], axis=1)
                first = _dot(h[:, :D // 2], w[:D // 2])
                y = _dot(h[:, D // 2:], w[D // 2:]) + first
                return y[:seg + n_mem, :E], y[:, E:2 * E], y[:, 2 * E:]
            if last:
                y = _dot(h, jnp.concatenate([head_w(hd, 1), head_w(hd, 2)], axis=1))
                return _dot(h[:seg], head_w(hd, 0)), y[:, :E], y[:, E:]
            y = _dot(h, jnp.concatenate([head_w(hd, 0), head_w(hd, 1)], axis=1))
            return y[:, :E], y[:, E:], _dot(h, head_w(hd, 2))

        def softmax_scores(q, k):
            sc = lax.dot_general(q, k, (((1,), (1,)), ((), ())), preferred_element_type=F32) * scale
            sc = jnp.where(allow[:seg + n_mem], sc, -1e9)
            p = jnp.exp(sc - jnp.max(sc, axis=-1, keepdims=True))
            return p / jnp.sum(p, axis=-1, keepdims=True)

        def out_proj(h0, h1, c):
            o = jnp.concatenate([head_out[hd] for hd in range(h0, h1)], axis=1)
            w = wo.at[c].bitcast(U32)[pl.ds(h0 * E // 2, (h1 - h0) * E // 2), :]
            return _dot(o, pltpu.bitcast(w, BF16))

        early = []
        for t in range(H + ND):
            if t < H:
                query[t], key[t], val[t] = project(t)
            else:
                early.append(out_proj(0, HEADS_EARLY, t - H))
            if 0 <= t - QK_LAG < H:
                hd = t - QK_LAG
                prob[hd] = softmax_scores(query.pop(hd), key.pop(hd))
            if 0 <= t - PV_LAG < H:
                hd = t - PV_LAG
                o = _dot(prob.pop(hd), val.pop(hd))
                head_out[hd] = o if last else jnp.concatenate([o[seg:], o[:seg]], axis=0)
        res = jnp.concatenate([out_proj(HEADS_EARLY, H, c) + early[c] for c in range(ND)], axis=1)

        gate = jnp.concatenate([gbuf[rows, :]] * ND, axis=1)
        obuf[rows, :] = (gate * res[n_mem:] + bbuf[rows, :]).astype(obuf.dtype)
        pltpu.make_async_copy(obuf.at[rows], out_hbm.at[rows], out_sem).start()
        return None if last else res[:M]

    def a_step(i, mem):
        for u in range(UNROLL):
            mem = segment(i * UNROLL + u, mem)
        return mem

    n_seg = S // seg
    n_steps = (n_seg - 1) // UNROLL
    mem = lax.fori_loop(0, n_steps, a_step, mem0[...].astype(F32))
    for s in range(n_steps * UNROLL, n_seg):
        mem = segment(s, mem, last=s == n_seg - 1)
    pltpu.make_async_copy(obuf, out_hbm, out_sem).wait()


@functools.partial(jax.jit, static_argnames=("A_seg_len",))
def pallas_gated_mix__memory_aug_recurrent_mem_tr__mixer_s_mlp__prompt_kernel(
    A_x: jax.Array,
    A_mem0: jax.Array,
    A_Wq: jax.Array,
    A_Wk: jax.Array,
    A_Wv: jax.Array,
    A_Wo: jax.Array,
    A_seg_len: int,
    B_x: jax.Array,
    B_w1: jax.Array,
    B_w2: jax.Array,
    B_w3: jax.Array,
    B_w4: jax.Array,
    gate_w: jax.Array,
):
    del B_x
    B, S, D = A_x.shape
    M = A_mem0.shape[1]
    _, H, E = A_Wq.shape
    F = B_w3.shape[1]
    seg = int(A_seg_len)
    nd = D // LANE
    dch = D // (S // B3_ROWS)
    assert B == 1 and E == LANE and D % (4 * LANE) == 0 and F % LANE == 0
    assert S % B3_ROWS == 0 and S > CUT2 + ROWS and S % seg == 0 and dch % 16 == 0
    assert seg % 16 == 0 and M % 8 == 0 and H % 16 == 0 and HEADS_EARLY + PV_LAG <= H and PV_LAG <= nd

    hbm = pl.BlockSpec(memory_space=pl.ANY)
    out = pl.pallas_call(
        functools.partial(_kernel, seg=seg, n_heads=H),
        out_shape=jax.ShapeDtypeStruct((S, D), A_x.dtype),
        in_specs=[hbm] * 11,
        out_specs=hbm,
        scratch_shapes=[
            pltpu.VMEM((S, D), BF16),
            pltpu.VMEM((M, D), BF16),
            pltpu.VMEM((nd, LANE), BF16),
            pltpu.VMEM((nd, D, LANE), BF16),
            pltpu.VMEM((nd, D, LANE), BF16),
            pltpu.VMEM((F // LANE, D, LANE), BF16),
            pltpu.VMEM((nd, F, LANE), BF16),
            pltpu.VMEM((nd, H * E, LANE), BF16),
            pltpu.VMEM(((3 * H + 8) * (D // 2 + HEAD_PAD), LANE), U32),
            pltpu.VMEM((2, 3, dch * H, LANE), BF16),
            pltpu.VMEM((nd, S + 2 * PAD, LANE), F32),
            pltpu.VMEM((S, D), BF16),
            pltpu.VMEM((S, D), F32),
            pltpu.VMEM((S, LANE), F32),
            pltpu.VMEM((S, D), A_x.dtype),
            pltpu.SemaphoreType.DMA((10 + nd,)),
            pltpu.SemaphoreType.DMA((2, 3)),
        ],
        compiler_params=pltpu.CompilerParams(vmem_limit_bytes=112 * 1024 * 1024),
    )(
        A_x.reshape(S, D), A_mem0.reshape(M, D),
        A_Wq.reshape(D * H, E), A_Wk.reshape(D * H, E), A_Wv.reshape(D * H, E),
        A_Wo.reshape(H * E, D),
        B_w1, B_w2, B_w3, B_w4, gate_w.reshape(nd, LANE),
    )
    return out.reshape(B, S, D)
```
